```python
import jax
import jax.numpy as jnp

def _softmax(x, axis=-1):
    return jax.nn.softmax(x, axis=axis)
def _gelu(x):
    return jax.nn.gelu(x, approximate=True)
def _silu(x):
    return jax.nn.silu(x)
def _sigmoid(x):
    return jax.nn.sigmoid(x)
def _layernorm(x, axis=-1, eps=1e-5):
    m = jnp.mean(x, axis=axis, keepdims=True)
    v = jnp.var(x, axis=axis, keepdims=True)
    return (x - m) / jnp.sqrt(v + eps)
def _scatter_add(tgt, idx, src, axis=0):
    return tgt.at[idx].add(src)
def _segment_sum(src, seg, n):
    return jax.ops.segment_sum(src, seg, n)
class _Rng:
    def __init__(self, key):
        self._k = key
    def _next(self):
        self._k, sub = jax.random.split(self._k)
        return sub
    def normal(self, shape):
        return jax.random.normal(self._next(), shape, dtype=jnp.bfloat16)
    def randint(self, lo, hi, shape):
        return jax.random.randint(self._next(), shape, lo, hi, dtype=jnp.int32)
    def uniform(self, shape, lo=0.0, hi=1.0):
        return jax.random.uniform(self._next(), shape, jnp.bfloat16, lo, hi)
    def permutation(self, n):
        return jax.random.permutation(self._next(), n)


kernel_name = 'standalone__adm_resblock__diffusion'

def setup_inputs():
    _rng = _Rng(jax.random.key(int.from_bytes(__import__("os").urandom(4), "little")))
    _w = (lambda a: (lambda t: t.astype(jnp.bfloat16) if jnp.issubdtype(t.dtype, jnp.floating) else t)(jnp.asarray(a)))
    B, C, HW, E = 2, 512, 64, 1152
    sc = (9.0 * C) ** -0.5
    return {
        "x": _w((lambda *s: _rng.normal(s) * 0.05)(B, C, HW, HW)),
        "t_emb": _w((lambda *s: _rng.normal(s) * 0.05)(B, E)),
        "g1": _w(1.0 + 0.1 * (lambda *s: _rng.normal(s) * 0.05)(C)),
        "be1": _w(0.1 * (lambda *s: _rng.normal(s) * 0.05)(C)),
        "w1": _w((lambda *s: _rng.normal(s) * 0.05)(C, C, 3, 3) * sc),
        "w_emb": _w((lambda *s: _rng.normal(s) * 0.05)(E, C) * (E ** -0.5)),
        "g2": _w(1.0 + 0.1 * (lambda *s: _rng.normal(s) * 0.05)(C)),
        "be2": _w(0.1 * (lambda *s: _rng.normal(s) * 0.05)(C)),
        "w2": _w((lambda *s: _rng.normal(s) * 0.05)(C, C, 3, 3) * sc),
    }

def reference(x, t_emb, g1, be1, w1, w_emb, g2, be2, w2):
    B, C, H, W = x.shape
    G, eps = 4, 1e-5
    def gn(z, gamma, beta):
        zr = z.reshape(B, G, (C // G) * H * W)
        mu = zr.mean(-1).reshape(B, G, 1)
        var = ((zr - mu) ** 2).mean(-1).reshape(B, G, 1)
        zn = ((zr - mu) / jnp.sqrt(var + eps)).reshape(B, C, H, W)
        return zn * gamma.reshape(1, C, 1, 1) + beta.reshape(1, C, 1, 1)
    def conv3(z, w):
        zp = jnp.pad(z, ((0, 0), (0, 0), (1, 1), (1, 1)))
        taps = [jnp.einsum("bchw,oc->bohw", zp[:, :, i:i+H, j:j+W], w[:, :, i, j]) for i in range(3) for j in range(3)]
        out = taps[0]
        for t in taps[1:]:
            out = out + t
        return out
    h = conv3(_silu(gn(x, g1, be1)), w1)
    emb = _silu(t_emb) @ w_emb
    h = h + emb.reshape(B, C, 1, 1)
    h = conv3(_silu(gn(h, g2, be2)), w2)
    return x + h
```

```python
import jax
import jax.numpy as jnp
from jax import lax
import jax.experimental.pallas as pl
import jax.experimental.pallas.tpu as pltpu

F32, BF16, U32 = jnp.float32, jnp.bfloat16, jnp.uint32
R2 = 2.0 ** 0.5
EPS = 1e-5
LANES = 128
NG = 4
HW = 64
NT = HW // 4
NPIX = HW * HW
SROWS = 72


def _cij(i, j):
    return R2 ** (3 - i - j) if (i + j) % 2 == 0 else 2.0 ** ((3 - i - j) // 2)


def _bt(p3m, p0, p1, p2, p3, p0n):
    t = p1 * 0.25
    er = p1 - p3
    e1 = p3 - t
    o1 = p2 - p0 * 0.25
    orr = p0 - p2
    e2 = er + er
    return [(p3m - t) - er, e1 + o1, e1 - o1, e2 + orr, e2 - orr, (p0n + orr) - p2 * 4.0]


def _gt(g0, g1, g2):
    a0, a1, a2 = g0 * (1.0 / 6.0), g1 * (R2 / 6.0), g2 * (1.0 / 6.0)
    s = a0 + a2
    e1, er = s + a2, s + a0
    return [g0, e1 + a1, e1 - a1, er + a1, er - a1, g2]


def _at(m0, m1, m2, m3, m4, m5):
    s1, d1, sr, dr = m1 + m2, m1 - m2, m3 + m4, m3 - m4
    return [(m0 + s1) + sr, (d1 + d1) + dr, s1 * 4.0 + sr, (d1 * 8.0 + dr) + m5]


def _unpack(w):
    return [pltpu.unpack_elementwise(w, index=i, packed_dtype=BF16, unpacked_dtype=F32) for i in range(2)]


def _pack(lo, hi):
    return pltpu.pack_elementwise([lo, hi], packed_dtype=BF16)


def _interleave(*streams):
    order = []
    for si, items in enumerate(streams):
        for k, f in enumerate(items):
            order.append(((k + 0.5) / len(items), si, f))
    order.sort(key=lambda e: e[:2])
    for _, _, f in order:
        f()


def _kernel(x_hbm, t_hbm, g1_hbm, be1_hbm, w1_hbm, we_hbm, g2_hbm, be2_hbm, w2_hbm, o_hbm,
            xs, ws, wes, ts, g1s, be1s, g2s, be2s, par, aff, V, U, M, S, Hs, xsem, wsem, psem, osem):
    xu = xs.bitcast(U32)
    wu = ws.bitcast(U32)

    def x_copy(b, g):
        return pltpu.make_async_copy(x_hbm.at[b, :, pl.ds(g * LANES, LANES)], xs.at[b, g], xsem.at[b, g])

    def w_copy(c, n, k):
        w_hbm = (w1_hbm, w2_hbm)[c]
        return pltpu.make_async_copy(
            w_hbm.at[:, pl.ds(n * LANES, LANES), pl.ds(k * LANES, LANES)],
            ws.at[c, k, :, pl.ds(n * LANES, LANES), :], wsem.at[c, n, k])

    def o_copy(b, g):
        return pltpu.make_async_copy(xs.at[b, g], o_hbm.at[b, :, pl.ds(g * LANES, LANES)], osem.at[b, g])

    small = [pltpu.make_async_copy(s, d, psem.at[i]) for i, (s, d) in enumerate(
        [(g1_hbm, g1s), (be1_hbm, be1s), (g2_hbm, g2s), (be2_hbm, be2s), (t_hbm, ts), (we_hbm, wes)])]

    def gn_finalize(slot, ssum, ssq, gamma, beta, shift):
        s1 = jnp.sum(ssum, axis=0, keepdims=True)
        s2 = jnp.sum(ssq, axis=0, keepdims=True)
        inv = 1.0 / (NPIX * LANES)
        mu = jnp.sum(s1 + shift * float(NPIX), axis=1, keepdims=True) * inv
        d = shift - mu
        var = jnp.sum(s2 + d * (2.0 * s1 + d * float(NPIX)), axis=1, keepdims=True) * inv
        scale = (0.5 * gamma) * lax.rsqrt(jnp.maximum(var, 0.0) + EPS)
        aff[slot, 0] = jnp.broadcast_to(scale, (8, LANES))
        aff[slot, 1] = jnp.broadcast_to(0.5 * beta + d * scale, (8, LANES))

    def prm(row, g):
        return par[row:row + 1, g * LANES:(g + 1) * LANES]

    def x_stats(b, g):
        acc = [jnp.zeros((8, LANES), F32) for _ in range(4)]

        def item(c):
            for r in range(16):
                lo, hi = _unpack(xu[b, g, pl.ds((c * 16 + r) * 8, 8), :])
                acc[0] += lo
                acc[1] += hi
                acc[2] += lo * lo
                acc[3] += hi * hi

        def fin():
            gn_finalize(b * NG + g, acc[0] + acc[1], acc[2] + acc[3], prm(0, g), prm(1, g),
                        jnp.zeros((1, LANES), F32))

        return [lambda c=c: item(c) for c in range(16)] + [fin]

    soff = {(0, 1): 0, (0, 0): 8, (3, 1): 24, (3, 0): 32, (1, 0): 40, (1, 1): 48, (2, 0): 56, (2, 1): 64}

    def in_transform(u, k):
        c, b = divmod(u, 2)
        slot = u * NG + k
        zero = jnp.zeros((8, LANES), F32)
        carry = {}

        def act(i, th, jp, e):
            if th >= NT:
                return [zero, zero]
            if c == 0:
                raw = _unpack(xu[b, k, pl.ds((4 * th + i) * 32 + 2 * e + jp, 8, stride=4), :])
            else:
                raw = [Hs[b, k, i, 2 * jp + q, pl.ds(th * NT + e, 8, stride=2), :] for q in range(2)]
            scale, bias = aff[slot, 0], aff[slot, 1]
            out = []
            for q in range(2):
                hz = raw[q] * scale + bias
                cz = _cij(i, 2 * jp + q)
                th_ = jnp.tanh(hz)
                out.append(hz * (th_ + 1.0) if cz == 1.0 else hz * (th_ * cz + cz))
            return out

        def col(chunk, jp, e):
            if chunk == 0:
                carry[jp, e] = ([zero, zero], act(0, 0, jp, e))
            for th in range(4 * chunk, 4 * chunk + 4):
                p3m, p0 = carry[jp, e]
                p1, p2, p3, p0n = act(1, th, jp, e), act(2, th, jp, e), act(3, th, jp, e), act(0, th + 1, jp, e)
                for q in range(2):
                    v = _bt(p3m[q], p0[q], p1[q], p2[q], p3[q], p0n[q])
                    for xi in range(6):
                        S[th, xi, pl.ds(soff[2 * jp + q, e], 8), :] = v[xi]
                carry[jp, e] = (p3, p0n)

        def row(th):
            for xi in range(6):
                p = {je: S[th, xi, pl.ds(o, 8), :] for je, o in soff.items()}
                p0n = S[th, xi, pl.ds(soff[0, 0] + 1, 8), :]
                p3m = S[th, xi, pl.ds(soff[3, 1] - 1, 8), :]
                ve = _bt(p3m, p[0, 0], p[1, 0], p[2, 0], p[3, 0], p[0, 1])
                vo = _bt(p[3, 0], p[0, 1], p[1, 1], p[2, 1], p[3, 1], p0n)
                for nu in range(6):
                    V[u % 2, xi * 6 + nu, k, pl.ds(th * 8, 8), :] = _pack(ve[nu], vo[nu])

        items = []
        for chunk in range(4):
            items += [lambda a=(chunk, jp, e): col(*a) for jp in range(2) for e in range(2)]
            items += [lambda th=th: row(th) for th in range(4 * chunk, 4 * chunk + 4)]
        return items

    def w_transform(c, n):
        def item(k, r):
            raw = [wu[c, k, t, pl.ds(n * 64 + r * 8, 8), :] for t in range(9)]
            g = [_unpack(w) for w in raw]
            half = []
            for q in range(2):
                cols = [_gt(g[l][q], g[3 + l][q], g[6 + l][q]) for l in range(3)]
                half.append([_gt(cols[0][xi], cols[1][xi], cols[2][xi]) for xi in range(6)])
            for xi in range(6):
                for nu in range(6):
                    if xi in (0, 5) and nu in (0, 5):
                        w = raw[(xi // 5) * 6 + (nu // 5) * 2]
                    else:
                        w = _pack(half[0][xi][nu], half[1][xi][nu])
                    U[n, xi * 6 + nu, k, pl.ds(r * 8, 8), :] = w

        return [lambda a=(k, r): item(*a) for k in range(NG) for r in range(8)]

    def matmuls(s):
        u, n = divmod(s, NG)

        def item(p):
            lhs = jnp.concatenate([pltpu.bitcast(V[u % 2, p, k], BF16) for k in range(NG)], axis=1)
            rhs = jnp.concatenate([pltpu.bitcast(U[n, p, k], BF16) for k in range(NG)], axis=1)
            M[s % 2, p] = lax.dot_general(lhs, rhs, (((1,), (1,)), ((), ())), preferred_element_type=F32)

        return [lambda p=p: item(p) for p in range(36)]

    def out_transform(s):
        u, n = divmod(s, NG)
        c, b = divmod(u, 2)
        acc = [jnp.zeros((8, LANES), F32) for _ in range(4)]

        def item(tv):
            rows = [_at(*[M[s % 2, xi * 6 + nu, pl.ds(tv * 8, 8), :] for nu in range(6)]) for xi in range(6)]
            for jp in range(2):
                z = [_at(*[rows[xi][2 * jp + q] for xi in range(6)]) for q in range(2)]
                for i in range(4):
                    y = [z[q][i] if _cij(i, 2 * jp + q) == 1.0 else z[q][i] * _cij(i, 2 * jp + q) for q in range(2)]
                    if c == 0:
                        for q in range(2):
                            Hs[b, n, i, 2 * jp + q, pl.ds(tv * 8, 8), :] = y[q]
                            acc[q] += y[q]
                            acc[2 + q] += y[q] * y[q]
                    else:
                        sl = pl.ds((4 * (tv // 2) + i) * 32 + (tv % 2) * 16 + jp, 8, stride=2)
                        lo, hi = _unpack(xu[b, n, sl, :])
                        xu[b, n, sl, :] = _pack(lo + y[0], hi + y[1])

        def fin():
            if c == 0:
                gn_finalize((u + 2) * NG + n, acc[0] + acc[1], acc[2] + acc[3], prm(2, n), prm(3, n), prm(4 + b, n))
            else:
                o_copy(b, n).start()

        return [lambda tv=tv: item(tv) for tv in range(2 * NT)] + [fin]

    x_copy(0, 0).start()
    for cp in small[:4]:
        cp.start()
    for g in range(1, NG):
        x_copy(0, g).start()
    for k in range(NG):
        w_copy(0, 0, k).start()
    for cp in small[4:]:
        cp.start()
    for n in range(NG):
        x_copy(1, n).start()
        if n + 1 < NG:
            for k in range(NG):
                w_copy(0, n + 1, k).start()
    for n in range(NG):
        for k in range(NG):
            w_copy(1, n, k).start()

    S[:, :, pl.ds(16, 8), :] = jnp.zeros((NT, 6, 8, LANES), F32)
    for i, (cp, ref) in enumerate(zip(small[:4], (g1s, be1s, g2s, be2s))):
        cp.wait()
        par[i:i + 1, :] = ref[...].astype(F32).reshape(1, NG * LANES)
    for g in range(NG):
        x_copy(0, g).wait()
        _interleave(x_stats(0, g))
        _interleave(in_transform(0, g))
    for k in range(NG):
        w_copy(0, 0, k).wait()
    for cp in small[4:]:
        cp.wait()
    x_copy(1, 0).wait()
    t = ts[...].astype(F32)
    t = (0.5 * t) * (jnp.tanh(0.5 * t) + 1.0)
    par[4:6, :] = jnp.dot(t.astype(BF16), wes[...], preferred_element_type=F32)
    _interleave(w_transform(0, 0), x_stats(1, 0))

    for s in range(4 * NG):
        u, n = divmod(s, NG)
        streams = [matmuls(s)]
        if s > 0:
            streams.append(out_transform(s - 1))
        if u < 3:
            streams.append(in_transform(u + 1, n))
        if s < NG - 1:
            x_copy(1, n + 1).wait()
            streams.append(x_stats(1, n + 1))
        wt = (0, s + 1) if s < NG - 1 else (1, s - 5) if 5 <= s < 5 + NG else None
        if wt is not None:
            for k in range(NG):
                w_copy(*wt, k).wait()
            streams.append(w_transform(*wt))
        _interleave(*streams)
    _interleave(out_transform(4 * NG - 1))
    for b in range(2):
        for g in range(NG):
            o_copy(b, g).wait()


@jax.jit
def pallas_standalone__adm_resblock__diffusion_kernel(
    x: jax.Array,
    t_emb: jax.Array,
    g1: jax.Array,
    be1: jax.Array,
    w1: jax.Array,
    w_emb: jax.Array,
    g2: jax.Array,
    be2: jax.Array,
    w2: jax.Array,
):
    B, C, H, W = x.shape
    E = t_emb.shape[1]
    assert (B, C, H, W) == (2, NG * LANES, HW, HW)
    xl = x.transpose(0, 2, 3, 1).reshape(B, NPIX, C)
    w1l = w1.transpose(2, 3, 0, 1).reshape(9, C, C)
    w2l = w2.transpose(2, 3, 0, 1).reshape(9, C, C)
    hbm = pl.BlockSpec(memory_space=pltpu.HBM)
    out = pl.pallas_call(
        _kernel,
        out_shape=jax.ShapeDtypeStruct((B, NPIX, C), x.dtype),
        in_specs=[hbm] * 9,
        out_specs=hbm,
        scratch_shapes=[
            pltpu.VMEM((B, NG, NPIX, LANES), BF16),
            pltpu.VMEM((2, NG, 9, C, LANES), BF16),
            pltpu.VMEM((E, C), BF16),
            pltpu.VMEM((B, E), BF16),
            pltpu.VMEM((C,), BF16),
            pltpu.VMEM((C,), BF16),
            pltpu.VMEM((C,), BF16),
            pltpu.VMEM((C,), BF16),
            pltpu.VMEM((8, C), F32),
            pltpu.VMEM((4 * NG, 2, 8, LANES), F32),
            pltpu.VMEM((2, 36, NG, NT * NT // 2, LANES), U32),
            pltpu.VMEM((NG, 36, NG, LANES // 2, LANES), U32),
            pltpu.VMEM((2, 36, NT * NT, LANES), F32),
            pltpu.VMEM((NT, 6, SROWS, LANES), F32),
            pltpu.VMEM((B, NG, 4, 4, NT * NT, LANES), F32),
            pltpu.SemaphoreType.DMA((B, NG)),
            pltpu.SemaphoreType.DMA((2, NG, NG)),
            pltpu.SemaphoreType.DMA((6,)),
            pltpu.SemaphoreType.DMA((B, NG)),
        ],
        compiler_params=pltpu.CompilerParams(vmem_limit_bytes=110 * 2 ** 20),
        name="adm_resblock",
    )(xl, t_emb, g1, be1, w1l, w_emb, g2, be2, w2l)
    return out.reshape(B, H, W, C).transpose(0, 3, 1, 2)
```

```python
import os, contextlib
import numpy as np
import jax
import jax.numpy as jnp
from jax import lax
import jax.experimental.pallas as pl
import jax.experimental.pallas.tpu as pltpu

F32, BF16, U32 = jnp.float32, jnp.bfloat16, jnp.uint32
R2 = 2.0 ** 0.5
EPS = 1e-5
LANES = 128
NG = 4
HW = 64
NT = HW // 4
NTILE = NT * NT
NPIX = HW * HW
SROWS = 72
PAD = 8
E = lambda k, d: type(d)(os.environ.get(k, d))
ONLY = [int(v) for v in os.environ.get('ONLY', '').split(',') if v]
FLAGS = {f: True for f in os.environ.get('FLAGS', '').split(',') if f}
scope = (lambda n: jax.named_scope(n)) if os.environ.get('SCOPES') else (lambda n: contextlib.nullcontext())
ALPHA = E('ALPHA', 0.995)
MERGE = [int(v) for v in E('MERGE', '6,8,14,15').split(',') if v]
NM = E('NM', 5)
TAILC = (128, 64, 64)


def _cij(i, j):
    return R2 ** (3 - i - j) if (i + j) % 2 == 0 else 2.0 ** ((3 - i - j) // 2)


def _bt(p3m, p0, p1, p2, p3, p0n):
    t = p1 * 0.25
    er = p1 - p3
    e1 = p3 - t
    o1 = p2 - p0 * 0.25
    orr = p0 - p2
    e2 = er + er
    return [(p3m - t) - er, e1 + o1, e1 - o1, e2 + orr, e2 - orr, (p0n + orr) - p2 * 4.0]


def _gt(g0, g1, g2, c0=1.0 / 6.0, c1=R2 / 6.0):
    a0, a1, a2 = g0 * c0, g1 * c1, g2 * c0
    s = a0 + a2
    e1, er = s + a2, s + a0
    return [g0, e1 + a1, e1 - a1, er + a1, er - a1, g2]


def _at_even(m0, m1, m2, m3, m4):
    s1, sr = m1 + m2, m3 + m4
    return (m0 + s1) + sr, s1 * 4.0 + sr


def _at_odd(m1, m2, m3, m4, m5):
    d1, dr = m1 - m2, m3 - m4
    return (d1 + d1) + dr, (d1 * 8.0 + dr) + m5


def _unpack(w):
    return [lax.bitcast_convert_type(w << 16, F32), lax.bitcast_convert_type(w & np.uint32(0xFFFF0000), F32)]


def _pack(lo, hi):
    lo, hi = [lax.bitcast_convert_type(v.astype(BF16).astype(F32), U32) for v in (lo, hi)]
    return (lo >> 16) | hi


def _accumulate(acc, i, s, q):
    acc[i] = s if acc[i] is None else acc[i] + s
    acc[2 + i] = q if acc[2 + i] is None else acc[2 + i] + q


def _merge(*streams):
    order = []
    for si, items in enumerate(streams):
        work, done = sum(c for _, _, c in items), 0
        for it in items:
            order.append((done / work, si, it))
            done += it[2]
    return [it for _, _, it in sorted(order, key=lambda e: e[:2])]


def _run(items):
    for f, _, _ in items:
        f()


def _overlap(dots, items):
    total = sum(rows for _, rows in dots)
    work = sum(c for _, _, c in items)
    done, issued, start, res = 0, 0, 0, None
    for f, gate, cost in items:
        t = int(done / work * ALPHA * total) // 8 * 8
        done += cost
        if gate is not None:
            while issued == 0 or t >= start + dots[issued - 1][1]:
                if issued:
                    start += dots[issued - 1][1]
                res = dots[issued][0]()
                issued += 1
            gate(res[t - start:t - start + 8])
        f()
    for f, _ in dots[issued:]:
        f()


def _kernel(x_hbm, t_hbm, g1_hbm, be1_hbm, w1_hbm, we_hbm, g2_hbm, be2_hbm, w2_hbm, o_hbm,
            xs, ob, ws, wes, ts, vecs, par, aff, cw, V, U, M, S, Hs, zs, xsem, cx, wsem, psem, osem):
    xu = xs.bitcast(U32)
    ou = ob.bitcast(U32)
    wu = ws.bitcast(U32)
    Vu = [v.bitcast(U32) for v in V]
    Uu = [v.bitcast(U32) for v in U]

    def x_copy(b, g):
        return pltpu.make_async_copy(x_hbm.at[b, :, pl.ds(g * LANES, LANES)], xs.at[b * NG + g, pl.ds(0, NPIX)], xsem.at[b, g])

    def x0_copy(q):
        rows = pl.ds(q * (NPIX // 4), NPIX // 4)
        return pltpu.make_async_copy(x_hbm.at[0, rows, pl.ds(0, LANES)], xs.at[0, rows], cx.at[q])

    def w_copy(c, n, k):
        return pltpu.make_async_copy(
            (w1_hbm, w2_hbm)[c].at[:, pl.ds(n * LANES, LANES), pl.ds(k * LANES, LANES)],
            ws.at[c * NG + k, :, pl.ds(n * LANES, LANES), :], wsem.at[c, n, k])

    def o_copy(b, g, r0=0, nr=NPIX, i=0):
        rows = pl.ds(r0, nr)
        return pltpu.make_async_copy(ob.at[b * NG + g, rows], o_hbm.at[b, rows, pl.ds(g * LANES, LANES)], osem.at[b * NG + g + i])

    small = [pltpu.make_async_copy(s, d, psem.at[i]) for i, (s, d) in enumerate(
        [(g1_hbm, vecs[0]), (be1_hbm, vecs[1]), (g2_hbm, vecs[2]), (be2_hbm, vecs[3]), (t_hbm, ts), (we_hbm, wes)])]

    for q in range(4):
        x0_copy(q).start()
        if q == 0:
            small[0].start()
            small[1].start()
    x_copy(0, 1).start()

    @pl.loop(0, 3)
    def _(i):
        zs[i] = i >> 2

    z0, z1, z2 = zs[0], zs[1], zs[2]

    def gate_u32(ref, idx):
        return lambda v: ref.__setitem__(idx, lax.bitcast_convert_type(v, U32))

    def gate(ref, idx):
        return lambda v: ref.__setitem__(idx, v)

    gate_x = gate_u32(xu, (z1, pl.ds(NPIX // 2, 8)))
    gate_w = gate_u32(wu, (z1, 0, pl.ds(NG * LANES // 2, 8)))
    gate_s = gate(S, (z1 + NT, 0, pl.ds(0, 8)))
    gate_c = gate(cw, z1 + 2)

    def gn_finalize(slot, acc, gamma, beta, shift):
        s1 = jnp.sum(acc[0] + acc[1], axis=0, keepdims=True)
        s2 = jnp.sum(acc[2] + acc[3], axis=0, keepdims=True)
        inv = 1.0 / (NPIX * LANES)
        mu = jnp.sum(s1 + shift * float(NPIX), axis=1, keepdims=True) * inv
        d = shift - mu
        var = jnp.sum(s2 + d * (2.0 * s1 + d * float(NPIX)), axis=1, keepdims=True) * inv
        scale = (0.5 * gamma) * lax.rsqrt(jnp.maximum(var, 0.0) + EPS)
        aff[slot][0] = jnp.broadcast_to(scale, (8, LANES))
        aff[slot][1] = jnp.broadcast_to(0.5 * beta + d * scale, (8, LANES))

    def x_stats(b, g):
        acc = [None] * 4

        def item(c):
            for r in range(8):
                lo, hi = _unpack(xu[b * NG + g, pl.ds((c * 8 + r) * 8, 8), :])
                _accumulate(acc, r & 1, lo + hi, lo * lo + hi * hi)

        def fin():
            gn_finalize(b * NG + g, acc, par[g, 0], par[g, 1], jnp.zeros((1, LANES), F32))

        return [(lambda c=c: item(c), gate_x, E('XCOST', 64)) for c in range(32)] + [(fin, None, 40)]

    soff = {(0, 1): 0, (0, 0): 8, (3, 1): 24, (3, 0): 32, (1, 0): 40, (1, 1): 48, (2, 0): 56, (2, 1): 64}

    def in_transform(c, b, k, t0=0, t1=NT):
        slot = (c * 2 + b) * NG + k
        zero = jnp.zeros((8, LANES), F32)
        carry = {}

        def act(i, th, jp, e):
            if th in (-1, NT):
                return [zero, zero]
            if c == 0:
                raw = _unpack(xu[b * NG + k, pl.ds((4 * th + i) * 32 + 2 * e + jp, 8, stride=4), :])
            else:
                raw = [Hs[b * NG + k][4 * i + 2 * jp + q, pl.ds(th * NT + 8 * e, 8), :] for q in range(2)]
            scale, bias = aff[slot][0], aff[slot][1]
            out = []
            for q in range(2):
                hz = raw[q] * scale + bias
                cz = _cij(i, 2 * jp + q)
                t = jnp.tanh(hz)
                out.append(hz * (t + 1.0) if cz == 1.0 else hz * (t * cz + cz))
            return out

        def col(th, jp, e):
            if th == t0:
                carry[jp, e] = (act(3, th - 1, jp, e), act(0, th, jp, e))
            p3m, p0 = carry[jp, e]
            p1, p2, p3, p0n = act(1, th, jp, e), act(2, th, jp, e), act(3, th, jp, e), act(0, th + 1, jp, e)
            for q in range(2):
                v = _bt(p3m[q], p0[q], p1[q], p2[q], p3[q], p0n[q])
                for xi in range(6):
                    S[z2 + th, xi, pl.ds(soff[2 * jp + q, e], 8), :] = v[xi]
            carry[jp, e] = (p3, p0n)

        def row(th, xi):
            p = {je: S[th, xi, pl.ds(o, 8), :] for je, o in soff.items()}
            p0n = S[th, xi, pl.ds(soff[0, 0] + 1, 8), :]
            p3m = S[th, xi, pl.ds(soff[3, 1] - 1, 8), :]
            ve = _bt(p3m, p[0, 0], p[1, 0], p[2, 0], p[3, 0], p[0, 1])
            vo = _bt(p[3, 0], p[0, 1], p[1, 1], p[2, 1], p[3, 1], p0n)
            for nu in range(6):
                V[b][xi * 6 + nu, k, pl.ds(th * 16, 8), :] = ve[nu].astype(BF16)
                V[b][xi * 6 + nu, k, pl.ds(th * 16 + 8, 8), :] = vo[nu].astype(BF16)

        src = gate_x if c == 0 else gate(Hs[b * NG + k], (z1, pl.ds(NTILE, 8)))
        cc = E('CCOST', 80) + (8 if c == 0 else 0)
        ch = min(E('CH', 8), t1 - t0)
        items = []
        for c0 in range(t0, t1, ch):
            items += [(lambda a=(th, jp, e): col(*a), src, cc) for jp in range(2) for e in range(2) for th in range(c0, c0 + ch)]
            items += [(lambda a=(th, xi): row(*a), gate_s, E('RCOST', 44)) for th in range(c0, c0 + ch) for xi in range(6)]
        return items

    def w_transform(c, n, ks=range(NG)):
        st = {}

        def put(k, r, q, xi, nu, v):
            U[n][xi * 6 + nu, k, pl.ds(r * 16 + q * 8, 8), :] = v.astype(BF16)

        def first(k, r, q):
            raw = [wu[c * NG + k, t, pl.ds(n * 64 + r * 8, 8), :] for t in range(9)]
            g = [pltpu.bitcast(w, BF16).astype(F32)[8 * q:8 * q + 8] for w in raw]
            st['cols'] = cols = [_gt(g[l], g[3 + l], g[6 + l]) for l in range(3)]
            if q == 0:
                for xi in (0, 5):
                    for nu in (0, 5):
                        Uu[n][xi * 6 + nu, k, pl.ds(r * 8, 8), :] = raw[(xi // 5) * 6 + (nu // 5) * 2]
            for xi in range(1, 5):
                put(k, r, q, xi, 0, cols[0][xi])
                put(k, r, q, xi, 5, cols[2][xi])

        def second(k, r, q, xis):
            cols = st['cols']
            c0, c1 = cw[0], cw[1]
            for xi in xis:
                u6 = _gt(cols[0][xi], cols[1][xi], cols[2][xi], c0, c1)
                for nu in range(1, 5):
                    put(k, r, q, xi, nu, u6[nu])

        wc = E('WCOST', 150) / 131
        items = []
        for k in ks:
            for r in range(8):
                for q in range(2):
                    items.append((lambda a=(k, r, q): first(*a), gate_w, 47 * wc))
                    items += [(lambda a=(k, r, q, g): second(*a), gate_c, 28 * wc) for g in ((0, 5), (1, 2), (3, 4))]
        return items

    def matmuls(s, dst, r0=0, nr=NTILE, d0=0, zv=0):
        u, n = divmod(s, NG)

        def item(p):
            lhs = [pltpu.bitcast(Vu[u & 1][p, k, pl.ds(r0 // 2, nr // 2), :], BF16) for k in range(NG)]
            rhs = [pltpu.bitcast(Uu[n][p, k], BF16) for k in range(NG)]
            r = lax.dot_general(jnp.concatenate(lhs, axis=1), jnp.concatenate(rhs, axis=1),
                                (((1,), (1,)), ((), ())), preferred_element_type=F32)
            dst[p, pl.ds(d0, nr), :] = r
            return r

        return [(lambda p=p: item(p), nr) for p in range(36)]

    def out_transform(s, src, r0=0, nr=NTILE, dma=0):
        c, b, n = s >> 3, (s >> 2) & 1, s & 3
        acc = [None] * 4
        rows = {}

        def first(d, odd, nus):
            for nu in nus:
                m = [src[z0 + xi * 6 + nu, pl.ds(d * 8, 8), :] for xi in range(odd, 5 + odd)]
                rows[nu] = (_at_odd if odd else _at_even)(*m)

        def second(d, odd):
            tv = r0 // 8 + d
            for q in range(2):
                i = odd + 2 * q
                m = [rows[nu][q] for nu in range(6)]
                (y0, y2), (y1, y3) = _at_even(*m[:5]), _at_odd(*m[1:])
                y = [z if _cij(i, j) == 1.0 else z * _cij(i, j) for j, z in enumerate((y0, y1, y2, y3))]
                if c == 0:
                    for j in range(4):
                        Hs[b * NG + n][4 * i + j, pl.ds(tv * 8, 8), :] = y[j]
                    _accumulate(acc, q, (y[0] + y[1]) + (y[2] + y[3]),
                                (y[0] * y[0] + y[1] * y[1]) + (y[2] * y[2] + y[3] * y[3]))
                else:
                    for jp in range(2):
                        sl = pl.ds((4 * (tv // 2) + i) * 32 + 2 * (tv % 2) + jp, 8, stride=4)
                        lo, hi = _unpack(xu[b * NG + n, sl, :])
                        ou[b * NG + n, sl, :] = _pack(lo + y[2 * jp], hi + y[2 * jp + 1])

        def fin():
            if c == 0:
                gn_finalize((2 + b) * NG + n, acc, par[n, 2], par[n, 3], par[n, 4 + b])
            else:
                o_copy(b, n, r0 * 16, nr * 16, dma).start()

        g = gate(src, (z1, pl.ds(src.shape[1] - 8, 8)))
        items = []
        for d in range(nr // 8):
            for odd in range(2):
                items += [(lambda a=(d, odd, nus): first(*a), g, E('O1COST', 21)) for nus in ((0, 1, 2), (3, 4, 5))]
                items += [(lambda a=(d, odd): second(*a), None, E('O2COST', 56) + E('O3', 16) * c)]
        return items + [(fin, None, 40)]

    def barrier():
        pl.loop(0, z1)(lambda i: zs.__setitem__(3, i))

    cw[0] = jnp.full((8, LANES), 1.0 / 6.0, F32)
    cw[1] = jnp.full((8, LANES), R2 / 6.0, F32)
    S[:, :, pl.ds(16, 8), :] = jnp.zeros((NT + 1, 6, 8, LANES), F32)

    def w_start(c, n, ks=range(NG)):
        for k in ks:
            w_copy(c, n, k).start()

    def w_wait(c, n, ks=range(NG)):
        for k in ks:
            w_copy(c, n, k).wait()

    H = NT // 2
    def load_vecs(rows):
        for i in rows:
            v = vecs[i][...].astype(F32).reshape(1, NG * LANES)
            for g in range(NG):
                par[g, i] = v[:, g * LANES:(g + 1) * LANES]

    if not ONLY:
        with scope('p_first'):
            st = x_stats(0, 0)
            for q in range(4):
                x0_copy(q).wait()
                if q == 1:
                    x_copy(0, 2).start()
                    w_start(0, 0, (0,))
                    x_copy(0, 3).start()
                    small[0].wait()
                    small[1].wait()
                    load_vecs((0, 1))
                _run(st[8 * q:8 * q + 8])
            _run(st[32:])
        with scope('p_g0'):
            _run(in_transform(0, 0, 0, 0, H + 4))
        with scope('p_g1'):
            x_copy(0, 1).wait()
            w_start(0, 0, (1, 2, 3))
            _run(x_stats(0, 1) + in_transform(0, 0, 1, 0, H))
        with scope('p_g2'):
            x_copy(0, 2).wait()
            w_start(0, 1)
            _run(x_stats(0, 2) + in_transform(0, 0, 2, 0, H))
            w_wait(0, 0, (0,))
            _run(w_transform(0, 0, (0,)))
        with scope('p_g3'):
            x_copy(0, 3).wait()
            w_start(0, 2)
            _run(x_stats(0, 3) + in_transform(0, 0, 3, 0, H))
            w_wait(0, 0, (1, 2, 3))
            _run(w_transform(0, 0, (1, 2, 3)))

    def embed():
        load_vecs((2, 3))
        t = ts[...].astype(F32)
        t = (0.5 * t) * (jnp.tanh(0.5 * t) + 1.0)
        emb = jnp.dot(t.astype(BF16), wes[...], preferred_element_type=F32)
        for n in range(NG):
            for b in range(2):
                par[n, 4 + b] = emb[b:b + 1, n * LANES:(n + 1) * LANES]

    MM = lambda s, *a: matmuls(s, M[s % NM], *a)
    OUT = lambda s: out_transform(s, M[s % NM])
    IN, WT, ST = in_transform, w_transform, x_stats
    T2 = NTILE // 2
    start = lambda *cps: [cp.start for cp in cps]
    wait = lambda *cps: [cp.wait for cp in cps]
    wc = lambda c, n: [w_copy(c, n, k) for k in range(NG)]
    plan = [
        lambda: (wait(*wc(0, 1)) + start(x_copy(1, 0)), MM(0, 0, T2), IN(0, 0, 0, H + 4, NT) + WT(0, 1)),
        lambda: (wait(*wc(0, 2)) + start(x_copy(1, 1), *wc(0, 3)), MM(1, 0, T2), IN(0, 0, 1, H, H + 4) + WT(0, 2)),
        lambda: (start(x_copy(1, 2), x_copy(1, 3), *small[2:]), MM(2, 0, T2), IN(0, 0, 1, H + 4, NT) + IN(0, 0, 2, H, NT) + IN(0, 0, 3, H, NT)),
        lambda: (wait(x_copy(1, 0), x_copy(1, 1), *wc(0, 3)) + start(*wc(1, 0), *wc(1, 1)),
                 MM(0, T2, T2, T2) + MM(1, T2, T2, T2), ST(1, 0) + WT(0, 3) + IN(0, 1, 0) + ST(1, 1)),
        lambda: (wait(x_copy(1, 2), x_copy(1, 3)) + start(*wc(1, 2), *wc(1, 3)), MM(2, T2, T2, T2) + MM(3),
                 ST(1, 2) + IN(0, 1, 1) + ST(1, 3) + IN(0, 1, 2) + IN(0, 1, 3)),
        lambda: (wait(*wc(1, 0), *wc(1, 1), *wc(1, 2), *wc(1, 3), *small[2:]) + [embed], MM(4), OUT(0) + OUT(1) + IN(1, 0, 0)),
        lambda: ([], MM(5), OUT(2) + OUT(3) + IN(1, 0, 1)),
        lambda: ([], MM(6), OUT(4) + IN(1, 0, 2) + WT(1, 0, (0, 1, 2))),
        lambda: ([], MM(7), OUT(5) + IN(1, 0, 3) + WT(1, 0, (3,)) + WT(1, 1, (0, 1))),
        lambda: ([], MM(8), OUT(6) + OUT(7) + WT(1, 1, (2, 3)) + WT(1, 2, (0, 1))),
        lambda: ([], MM(9), OUT(8) + IN(1, 1, 0) + WT(1, 2, (2, 3))),
        lambda: ([], MM(10), IN(1, 1, 1) + WT(1, 3) + IN(1, 1, 2, 0, H)),
        lambda: ([], MM(11), OUT(9) + IN(1, 1, 2, H, NT) + IN(1, 1, 3)),
        lambda: ([], MM(12), OUT(10) + OUT(11)),
        lambda: ([], MM(13), OUT(12)),
        lambda: ([], MM(14), OUT(13)),
    ]
    for i, blk in enumerate(plan):
        if ONLY and i not in ONLY:
            continue
        dmas, dots, items = blk()
        if i not in MERGE:
            with scope('bar%02d' % i):
                barrier()
        if not ONLY:
            with scope('dma%02d' % i):
                for f in dmas:
                    f()
        with scope('blk%02d' % i):
            _overlap(dots, items)
    if not ONLY or 16 in ONLY:
        if 16 not in MERGE:
            barrier()
        with scope('blk16'):
            items, r0 = OUT(14), 0
            for i, nr in enumerate(TAILC):
                _overlap(matmuls(15, M[(15 + i) % NM], r0, nr), items)
                items = out_transform(15, M[(15 + i) % NM], r0, nr, i)
                r0 += nr
            _run(items)

    if not ONLY:
        with scope('e_dma'):
            for i in range(2 * NG - 1):
                o_copy(*divmod(i, NG)).wait()
            r0 = 0
            for i, nr in enumerate(TAILC):
                o_copy(1, NG - 1, r0 * 16, nr * 16, i).wait()
                r0 += nr
    else:
        barrier()
        acc = jnp.zeros((8, LANES), F32)
        for r in Vu + Uu:
            acc += lax.bitcast_convert_type(r[z0, 0, 0:8, :], F32)
        for r in M + Hs:
            acc += r[z0, 0:8, :]
        for r in aff:
            acc += r[z0]
        ob[0, 0:8, :] = acc.astype(BF16)
        o_copy(0, 0).start()
        o_copy(0, 0).wait()


@jax.jit
def pallas_standalone__adm_resblock__diffusion_kernel(x, t_emb, g1, be1, w1, w_emb, g2, be2, w2):
    B, C, H, W = x.shape
    E_ = t_emb.shape[1]
    xl = x.transpose(0, 2, 3, 1).reshape(B, NPIX, C)
    w1l = w1.transpose(2, 3, 0, 1).reshape(9, C, C)
    w2l = w2.transpose(2, 3, 0, 1).reshape(9, C, C)
    hbm = pl.BlockSpec(memory_space=pltpu.HBM)
    out = pl.pallas_call(
        _kernel,
        out_shape=jax.ShapeDtypeStruct((B, NPIX, C), x.dtype),
        in_specs=[hbm] * 9,
        out_specs=hbm,
        scratch_shapes=[
            pltpu.VMEM((B * NG, NPIX + 16, LANES), BF16),
            pltpu.VMEM((B * NG, NPIX, LANES), BF16),
            pltpu.VMEM((2 * NG, 9, C + 16, LANES), BF16),
            pltpu.VMEM((E_, C), BF16),
            pltpu.VMEM((B, E_), BF16),
            [pltpu.VMEM((C,), BF16)] * 4,
            pltpu.VMEM((NG, 6, 1, LANES), F32),
            [pltpu.VMEM((2, 8, LANES), F32)] * (4 * NG),
            pltpu.VMEM((3, 8, LANES), F32),
            [pltpu.VMEM((36, NG, NTILE, LANES), BF16)] * 2,
            [pltpu.VMEM((36, NG, LANES, LANES), BF16)] * NG,
            [pltpu.VMEM((36, NTILE + PAD, LANES), F32)] * NM,
            pltpu.VMEM((NT + 1, 6, SROWS, LANES), F32),
            [pltpu.VMEM((16, NTILE + PAD, LANES), F32)] * (B * NG),
            pltpu.SMEM((4,), jnp.int32),
            pltpu.SemaphoreType.DMA((B, NG)),
            pltpu.SemaphoreType.DMA((4,)),
            pltpu.SemaphoreType.DMA((2, NG, NG)),
            pltpu.SemaphoreType.DMA((6,)),
            pltpu.SemaphoreType.DMA((B * NG + len(TAILC),)),
        ],
        compiler_params=pltpu.CompilerParams(vmem_limit_bytes=118 * 2 ** 20, flags=FLAGS or None, disable_bounds_checks=bool(E('NOBC', 1))),
        name="adm_resblock",
    )(xl, t_emb, g1, be1, w1l, w_emb, g2, be2, w2l)
    return out.reshape(B, H, W, C).transpose(0, 3, 1, 2)
```

```python
import numpy as np
import jax
import jax.numpy as jnp
from jax import lax
import jax.experimental.pallas as pl
import jax.experimental.pallas.tpu as pltpu

F32, BF16, U32 = jnp.float32, jnp.bfloat16, jnp.uint32
R2 = 2.0 ** 0.5
EPS = 1e-5
LANES = 128
NB = 2
NG = 4
HW = 64
NT = HW // 4
NTILE = NT * NT
NPIX = HW * HW
NPOS = 36
NM = 6
PAD = 8
TAIL = (128, 64, 64)

SOFF = {(0, 1): 0, (0, 0): 8, (3, 1): 24, (3, 0): 32, (1, 0): 40, (1, 1): 48, (2, 0): 56, (2, 1): 64}
SROWS = 72


def _phase_scale(i, j):
    return R2 ** (3 - i - j) if (i + j) % 2 == 0 else 2.0 ** ((3 - i - j) // 2)


def _bt(p3m, p0, p1, p2, p3, p0n):
    t = p1 * 0.25
    er = p1 - p3
    e1 = p3 - t
    o1 = p2 - p0 * 0.25
    orr = p0 - p2
    e2 = er + er
    return [(p3m - t) - er, e1 + o1, e1 - o1, e2 + orr, e2 - orr, (p0n + orr) - p2 * 4.0]


def _gt(g0, g1, g2, c0=1.0 / 6.0, c1=R2 / 6.0):
    a0, a1, a2 = g0 * c0, g1 * c1, g2 * c0
    s = a0 + a2
    e1, er = s + a2, s + a0
    return [g0, e1 + a1, e1 - a1, er + a1, er - a1, g2]


def _at_even(m0, m1, m2, m3, m4):
    s1, sr = m1 + m2, m3 + m4
    return (m0 + s1) + sr, s1 * 4.0 + sr


def _at_odd(m1, m2, m3, m4, m5):
    d1, dr = m1 - m2, m3 - m4
    return (d1 + d1) + dr, (d1 * 8.0 + dr) + m5


def _unpack(w):
    return [lax.bitcast_convert_type(w << 16, F32), lax.bitcast_convert_type(w & np.uint32(0xFFFF0000), F32)]


def _pack(lo, hi):
    lo, hi = [lax.bitcast_convert_type(v.astype(BF16).astype(F32), U32) for v in (lo, hi)]
    return (lo >> 16) | hi


def _accumulate(acc, i, s, q):
    acc[i] = s if acc[i] is None else acc[i] + s
    acc[2 + i] = q if acc[2 + i] is None else acc[2 + i] + q


def _run(items):
    for f, _, _ in items:
        f()


def _overlap(dots, items):
    total = sum(rows for _, rows in dots)
    work = sum(cost for _, _, cost in items)
    done, issued, start, res = 0, 0, 0, None
    for f, gate, cost in items:
        t = int(done / work * 0.995 * total) // 8 * 8
        done += cost
        if gate is not None:
            while issued == 0 or t >= start + dots[issued - 1][1]:
                if issued:
                    start += dots[issued - 1][1]
                res = dots[issued][0]()
                issued += 1
            gate(res[t - start:t - start + 8])
        f()
    for f, _ in dots[issued:]:
        f()


def _kernel(x_hbm, t_hbm, g1_hbm, be1_hbm, w1_hbm, we_hbm, g2_hbm, be2_hbm, w2_hbm, o_hbm,
            xs, ob, ws, wes, ts, vecs, par, aff, cw, V, U, M, S, Hs, zs, sem):
    xu, ou, wu = xs.bitcast(U32), ob.bitcast(U32), ws.bitcast(U32)
    Vu, Uu = [v.bitcast(U32) for v in V], [u.bitcast(U32) for u in U]
    lo, hi, every = (0, 1), (2, 3), range(NG)
    slab = lambda g: pl.ds(g * LANES, LANES)

    def x_copy(b, g, r0=0, nr=NPIX):
        rows = pl.ds(r0, nr)
        return [(x_hbm.at[b, rows, slab(g)], xs.at[b * NG + g, rows])]

    def w_copy(c, ns, ks):
        w_hbm = (w1_hbm, w2_hbm)[c]
        return [(w_hbm.at[:, slab(n), slab(k)], ws.at[c * NG + k, :, slab(n), :]) for n in ns for k in ks]

    early = 3 * NPIX // 4
    loads = dict(
        w0=w_copy(0, (0,), lo), w1=w_copy(0, (1,), lo),
        x0a=[(g1_hbm, vecs[0]), (be1_hbm, vecs[1])] + x_copy(0, 0, 0, early), x0b=x_copy(0, 0, early, NPIX - early),
        x1a=x_copy(0, 1, 0, early), x1b=x_copy(0, 1, early, NPIX - early),
        b0=[(g2_hbm, vecs[2]), (be2_hbm, vecs[3]), (t_hbm, ts)],
        b1=x_copy(0, 2) + w_copy(0, hi, lo),
        b2=x_copy(0, 3) + w_copy(0, lo, hi),
        b3=w_copy(0, hi, hi) + x_copy(1, 0) + x_copy(1, 1) + [(we_hbm, wes)],
        b4=x_copy(1, 2) + x_copy(1, 3),
        b5=w_copy(1, every, every))
    osem = sem.at[len(loads)]

    def copies(name):
        return [pltpu.make_async_copy(src, dst, sem.at[list(loads).index(name)]) for src, dst in loads[name]]

    def start(*names):
        for name in names:
            for cp in copies(name):
                cp.start()

    def wait(name):
        for cp in copies(name):
            cp.wait()

    def write_out(b, g, r0, nr):
        rows = pl.ds(r0, nr)
        pltpu.make_async_copy(ob.at[b * NG + g, rows], o_hbm.at[b, rows, slab(g)], osem).start()

    start("w0", "w1", "x0a", "x0b", "x1a", "x1b")

    @pl.loop(0, 3)
    def _(i):
        zs[i] = i >> 2

    z0, z1 = zs[0], zs[1]

    def gate(ref, idx):
        def put(v):
            ref[idx] = v if ref.dtype == F32 else lax.bitcast_convert_type(v, U32)
        return put

    gate_x = gate(xu, (z1, pl.ds(NPIX // 2, 8)))
    gate_w = gate(wu, (z1, 0, pl.ds(NG * LANES // 2, 8)))
    gate_s = gate(S, (z1 + NT, 0, pl.ds(0, 8)))
    gate_c = gate(cw, z1 + 2)

    def new_block():
        @pl.loop(0, z1)
        def _(i):
            zs[2] = i

    def reload():
        for ref in Vu[:1] + Uu:
            ref[z1 + NPOS, 0, 0:8, :] = jnp.zeros((8, LANES), U32)

    def load_vecs(rows):
        for r in rows:
            v = vecs[r][...].astype(F32).reshape(1, NG * LANES)
            for g in every:
                par[g, r] = v[:, g * LANES:(g + 1) * LANES]

    def embed():
        load_vecs(hi)
        t = 0.5 * ts[...].astype(F32)
        emb = jnp.dot((t * (jnp.tanh(t) + 1.0)).astype(BF16), wes[...], preferred_element_type=F32)
        for g in every:
            for b in range(NB):
                par[g, 4 + b] = emb[b:b + 1, g * LANES:(g + 1) * LANES]

    def gn_finalize(slot, acc, gamma, beta, shift):
        s1 = jnp.sum(acc[0] + acc[1], axis=0, keepdims=True)
        s2 = jnp.sum(acc[2] + acc[3], axis=0, keepdims=True)
        inv = 1.0 / (NPIX * LANES)
        mu = jnp.sum(s1 + shift * float(NPIX), axis=1, keepdims=True) * inv
        d = shift - mu
        var = jnp.sum(s2 + d * (2.0 * s1 + d * float(NPIX)), axis=1, keepdims=True) * inv
        scale = (0.5 * gamma) * lax.rsqrt(jnp.maximum(var, 0.0) + EPS)
        aff[slot][0] = jnp.broadcast_to(scale, (8, LANES))
        aff[slot][1] = jnp.broadcast_to(0.5 * beta + d * scale, (8, LANES))

    def x_stats(b, g):
        acc = [None] * 4

        def item(c):
            for r in range(8):
                u, v = _unpack(xu[b * NG + g, pl.ds((c * 8 + r) * 8, 8), :])
                _accumulate(acc, r & 1, u + v, u * u + v * v)

        def fin():
            gn_finalize(b * NG + g, acc, par[g, 0], par[g, 1], jnp.zeros((1, LANES), F32))

        return [(lambda c=c: item(c), gate_x, 64) for c in range(32)] + [(fin, None, 40)]

    def in_transform(c, b, k, t0=0, t1=NT):
        slot = (c * NB + b) * NG + k
        held = {}

        def act(i, th, jp, e):
            if th in (-1, NT):
                return [jnp.zeros((8, LANES), F32)] * 2
            if c == 0:
                raw = _unpack(xu[b * NG + k, pl.ds((4 * th + i) * 32 + 2 * e + jp, 8, stride=4), :])
            else:
                raw = [Hs[b * NG + k][4 * i + 2 * jp + q, pl.ds(th * NT + 8 * e, 8), :] for q in range(2)]
            scale, bias = aff[slot][0], aff[slot][1]
            out = []
            for q in range(2):
                hz = raw[q] * scale + bias
                cz = _phase_scale(i, 2 * jp + q)
                t = jnp.tanh(hz)
                out.append(hz * (t + 1.0) if cz == 1.0 else hz * (t * cz + cz))
            return out

        def activate(th, jp, e):
            if th == t0:
                held[jp, e] = (act(3, th - 1, jp, e), act(0, th, jp, e))
            held["new"] = [act(i, th, jp, e) for i in (1, 2, 3)]

        def along_h(th, jp, e):
            (p3m, p0), (p1, p2, p3), p0n = held[jp, e], held["new"], act(0, th + 1, jp, e)
            for q in range(2):
                v = _bt(p3m[q], p0[q], p1[q], p2[q], p3[q], p0n[q])
                for xi in range(6):
                    S[th, xi, pl.ds(SOFF[2 * jp + q, e], 8), :] = v[xi]
            held[jp, e] = (p3, p0n)

        def along_w(th, xi):
            p = {je: S[th, xi, pl.ds(o, 8), :] for je, o in SOFF.items()}
            p0n = S[th, xi, pl.ds(SOFF[0, 0] + 1, 8), :]
            p3m = S[th, xi, pl.ds(SOFF[3, 1] - 1, 8), :]
            even = _bt(p3m, p[0, 0], p[1, 0], p[2, 0], p[3, 0], p[0, 1])
            odd = _bt(p[3, 0], p[0, 1], p[1, 1], p[2, 1], p[3, 1], p0n)
            for nu in range(6):
                V[b][xi * 6 + nu, k, pl.ds(th * NT, 8), :] = even[nu].astype(BF16)
                V[b][xi * 6 + nu, k, pl.ds(th * NT + 8, 8), :] = odd[nu].astype(BF16)

        src = gate_x if c == 0 else gate(Hs[b * NG + k], (z1, pl.ds(NTILE, 8)))
        items = []
        for c0 in range(t0, t1, 4):
            for jp in range(2):
                for e in range(2):
                    for th in range(c0, c0 + 4):
                        items.append((lambda a=(th, jp, e): activate(*a), src, (33 if c else 39) + 22 * (th == t0)))
                        items.append((lambda a=(th, jp, e): along_h(*a), src, 45 if c else 47))
            items += [(lambda a=(th, xi): along_w(*a), gate_s, 48) for th in range(c0, c0 + 4) for xi in range(6)]
        return items

    def w_transform(c, n, ks=every):
        held = {}

        def put(k, r, q, xi, nu, v):
            U[n][xi * 6 + nu, k, pl.ds(r * 16 + q * 8, 8), :] = v.astype(BF16)

        def along_h(k, r, q):
            raw = [wu[c * NG + k, t, pl.ds(n * 64 + r * 8, 8), :] for t in range(9)]
            g = [pltpu.bitcast(w, BF16).astype(F32)[8 * q:8 * q + 8] for w in raw]
            held["cols"] = cols = [_gt(g[l], g[3 + l], g[6 + l]) for l in range(3)]
            if q == 0:
                for xi in (0, 5):
                    for nu in (0, 5):
                        Uu[n][xi * 6 + nu, k, pl.ds(r * 8, 8), :] = raw[(xi // 5) * 6 + (nu // 5) * 2]
            for xi in range(1, 5):
                put(k, r, q, xi, 0, cols[0][xi])
                put(k, r, q, xi, 5, cols[2][xi])

        def along_w(k, r, q, xis):
            cols = held["cols"]
            c0, c1 = cw[0], cw[1]
            for xi in xis:
                u = _gt(cols[0][xi], cols[1][xi], cols[2][xi], c0, c1)
                for nu in range(1, 5):
                    put(k, r, q, xi, nu, u[nu])

        items = []
        for k in ks:
            for r in range(8):
                for q in range(2):
                    items.append((lambda a=(k, r, q): along_h(*a), gate_w, 55.25))
                    items += [(lambda a=(k, r, q, xis): along_w(*a), gate_c, 32.9) for xis in ((0, 5), (1, 2), (3, 4))]
        return items

    def nt_dot(lhs, rhs):
        return lax.dot_general(lhs, rhs, (((1,), (1,)), ((), ())), preferred_element_type=F32)

    def operand(ref, p, ks, rows=slice(None)):
        return jnp.concatenate([pltpu.bitcast(ref[p, k, rows, :], BF16) for k in ks], axis=1)

    def matmuls(s, r0=0, nr=NTILE, dst=None):
        def item(p):
            r = nt_dot(operand(Vu[s >> 2 & 1], p, every, pl.ds(r0 // 2, nr // 2)), operand(Uu[s & 3], p, every))
            M[s % NM if dst is None else dst][p, pl.ds(r0, nr), :] = r
            return r

        return [(lambda p=p: item(p), nr) for p in range(NPOS)]

    def matmuls_half(ns, ks, r0=0, nr=NTILE):
        def item(p):
            r = nt_dot(operand(Vu[0], p, ks, pl.ds(r0 // 2, nr // 2)),
                       jnp.concatenate([operand(Uu[n], p, ks) for n in ns], axis=0))
            for i, n in enumerate(ns):
                part = r[:, i * LANES:(i + 1) * LANES]
                if ks[0]:
                    part = part + M[n][p, pl.ds(r0, nr), :]
                M[n][p, pl.ds(r0, nr), :] = part
            return part

        return [(lambda p=p: item(p), nr) for p in range(NPOS)]

    def out_transform(s, r0=0, nr=NTILE, src=None, piece=None):
        c, b, n = s >> 3, s >> 2 & 1, s & 3
        src = M[s % NM if src is None else src]
        piece = piece or nr
        acc, held = [None] * 4, {}

        def along_h(tv, odd, nus):
            for nu in nus:
                m = [src[z0 + xi * 6 + nu, pl.ds(tv * 8, 8), :] for xi in range(odd, 5 + odd)]
                held[nu] = (_at_odd if odd else _at_even)(*m)

        def along_w(tv, odd):
            for q in range(2):
                i = odd + 2 * q
                m = [held[nu][q] for nu in range(6)]
                (y0, y2), (y1, y3) = _at_even(*m[:5]), _at_odd(*m[1:])
                y = [z if _phase_scale(i, j) == 1.0 else z * _phase_scale(i, j) for j, z in enumerate((y0, y1, y2, y3))]
                if c == 0:
                    for j in range(4):
                        Hs[b * NG + n][4 * i + j, pl.ds(tv * 8, 8), :] = y[j]
                    _accumulate(acc, q, (y[0] + y[1]) + (y[2] + y[3]),
                                (y[0] * y[0] + y[1] * y[1]) + (y[2] * y[2] + y[3] * y[3]))
                else:
                    for jp in range(2):
                        sl = pl.ds((4 * (tv // 2) + i) * 32 + 2 * (tv % 2) + jp, 8, stride=4)
                        u, v = _unpack(xu[b * NG + n, sl, :])
                        ou[b * NG + n, sl, :] = _pack(u + y[2 * jp], v + y[2 * jp + 1])

        def fin(end):
            if c == 0:
                gn_finalize((NB + b) * NG + n, acc, par[n, 2], par[n, 3], par[n, 4 + b])
            else:
                write_out(b, n, (end - piece) * 16, piece * 16)

        g = gate(src, (z1, pl.ds(NTILE, 8)))
        items = []
        for tv in range(r0 // 8, (r0 + nr) // 8):
            for odd in range(2):
                items += [(lambda a=(tv, odd, nus): along_h(*a), g, 21) for nus in ((0, 1, 2), (3, 4, 5))]
                items += [(lambda a=(tv, odd): along_w(*a), None, 72 if c else 56)]
            if (tv * 8 + 8 - r0) % piece == 0:
                items.append((lambda end=tv * 8 + 8: fin(end), None, 40))
        return items

    ST, IN, WT, MM, MH, OUT = x_stats, in_transform, w_transform, matmuls, matmuls_half, out_transform
    H, T2 = NT // 2, NTILE // 2

    cw[0] = jnp.full((8, LANES), 1.0 / 6.0, F32)
    cw[1] = jnp.full((8, LANES), R2 / 6.0, F32)
    S[:, :, pl.ds(16, 8), :] = jnp.zeros((NT + 1, 6, 8, LANES), F32)

    wait("w0")
    _run(WT(0, 0, lo))
    wait("w1")
    _run(WT(0, 1, lo))
    wait("x0a")
    start("b0", "b1")
    load_vecs(lo)
    stats = ST(0, 0)
    _run(stats[:24])
    wait("x0b")
    first = IN(0, 0, 0, 0, H)
    _run(stats[24:] + first[:-24])
    stats = ST(0, 1)
    wait("x1a")
    _run(stats[:24])
    wait("x1b")
    start("b2")
    _run(stats[24:] + first[-24:] + IN(0, 0, 1, 0, H))

    wait("b0")
    _overlap(MH(lo, lo, 0, T2), IN(0, 0, 0, H, NT) + IN(0, 0, 1, H, NT))
    reload()
    wait("b1")
    start("b3")
    _overlap(MH(lo, lo, T2, T2), ST(0, 2) + WT(0, 2, lo) + WT(0, 3, lo))
    reload()
    wait("b2")
    start("b4")
    _overlap(MH(hi, lo), ST(0, 3) + WT(0, 0, hi) + IN(0, 0, 2, 0, H) + IN(0, 0, 3, 0, H) + WT(0, 1, hi))

    new_block()
    wait("b3")
    start("b5")
    _overlap(MH(lo, hi, 0, T2), [(embed, None, 1)] + ST(1, 0) + IN(0, 0, 2, H, NT) + IN(0, 0, 3, H, NT))
    _overlap(MH(lo, hi, T2, T2), ST(1, 1) + WT(0, 2, hi) + WT(0, 3, hi))

    new_block()
    wait("b4")
    out0, out2 = OUT(0), OUT(2)
    mid = len(out0) // 2
    _overlap(MH(hi, hi), sum([ST(1, 2), ST(1, 3)] + [IN(0, 1, k, 0, H) for k in every], []))
    _overlap(MM(4, 0, T2) + MM(5, 0, T2), sum([IN(0, 1, k, H, NT) for k in every], []) + out0[:mid])

    new_block()
    wait("b5")
    _overlap(MM(4, T2, T2) + MM(5, T2, T2), out0[mid:] + OUT(1) + IN(1, 0, 0) + out2[:mid])
    _overlap(MM(6), out2[mid:] + IN(1, 0, 1) + IN(1, 0, 2, 0, H) + WT(1, 0, (0, 1, 2)))

    new_block()
    _overlap(MM(7), OUT(3) + IN(1, 0, 2, H, NT) + IN(1, 0, 3) + WT(1, 0, (3,)))
    _overlap(MM(8), OUT(4) + OUT(5) + WT(1, 1))

    new_block()
    _overlap(MM(9), IN(1, 1, 0) + IN(1, 1, 1, 0, H) + WT(1, 2))
    _overlap(MM(10), OUT(6) + IN(1, 1, 1, H, NT) + IN(1, 1, 2, 0, 4) + WT(1, 3))

    new_block()
    _overlap(MM(11), OUT(7) + IN(1, 1, 2, 4, NT) + IN(1, 1, 3))
    _overlap(MM(12), OUT(8) + OUT(9))
    dots, items = MM(13), OUT(10) + OUT(11)
    cut = 5 * len(items) // 12
    _overlap(dots[:15], items[:cut])

    new_block()
    _overlap(dots[15:], items[cut:])
    _overlap(MM(14), OUT(12) + OUT(13))
    items, r0 = OUT(14), 0
    for i, nr in enumerate(TAIL):
        _overlap(MM(15, r0, nr, (15 + i) % NM), items)
        items = OUT(15, r0, nr, (15 + i) % NM, NT if i == len(TAIL) - 1 else None)
        r0 += nr
    _run(items)
    pltpu.make_async_copy(ob, ob, osem).wait()


@jax.jit
def pallas_standalone__adm_resblock__diffusion_kernel(
    x: jax.Array,
    t_emb: jax.Array,
    g1: jax.Array,
    be1: jax.Array,
    w1: jax.Array,
    w_emb: jax.Array,
    g2: jax.Array,
    be2: jax.Array,
    w2: jax.Array,
):
    B, C, H, W = x.shape
    E = t_emb.shape[1]
    assert (B, C, H, W) == (NB, NG * LANES, HW, HW)
    xl = x.transpose(0, 2, 3, 1).reshape(B, NPIX, C)
    w1l = w1.transpose(2, 3, 0, 1).reshape(9, C, C)
    w2l = w2.transpose(2, 3, 0, 1).reshape(9, C, C)
    hbm = pl.BlockSpec(memory_space=pltpu.HBM)
    out = pl.pallas_call(
        _kernel,
        out_shape=jax.ShapeDtypeStruct((B, NPIX, C), x.dtype),
        in_specs=[hbm] * 9,
        out_specs=hbm,
        scratch_shapes=[
            pltpu.VMEM((B * NG, NPIX + 2 * PAD, LANES), BF16),
            pltpu.VMEM((B * NG, NPIX, LANES), BF16),
            pltpu.VMEM((2 * NG, 9, C + 2 * PAD, LANES), BF16),
            pltpu.VMEM((E, C), BF16),
            pltpu.VMEM((B, E), BF16),
            [pltpu.VMEM((C,), BF16)] * 4,
            pltpu.VMEM((NG, 4 + B, 1, LANES), F32),
            [pltpu.VMEM((2, 8, LANES), F32)] * (2 * B * NG),
            pltpu.VMEM((3, 8, LANES), F32),
            [pltpu.VMEM((NPOS + 1, NG, NTILE, LANES), BF16)] * B,
            [pltpu.VMEM((NPOS + 1, NG, LANES, LANES), BF16)] * NG,
            [pltpu.VMEM((NPOS, NTILE + PAD, LANES), F32)] * NM,
            pltpu.VMEM((NT + 1, 6, SROWS, LANES), F32),
            [pltpu.VMEM((16, NTILE + PAD, LANES), F32)] * (B * NG),
            pltpu.SMEM((3,), jnp.int32),
            pltpu.SemaphoreType.DMA((13,)),
        ],
        compiler_params=pltpu.CompilerParams(vmem_limit_bytes=124 * 2 ** 20),
        name="adm_resblock",
    )(xl, t_emb, g1, be1, w1l, w_emb, g2, be2, w2l)
    return out.reshape(B, H, W, C).transpose(0, 3, 1, 2)
```

```python
import numpy as np
import jax
import jax.numpy as jnp
from jax import lax
import jax.experimental.pallas as pl
import jax.experimental.pallas.tpu as pltpu

F32, BF16, U32 = jnp.float32, jnp.bfloat16, jnp.uint32
R2 = 2.0 ** 0.5
EPS = 1e-5
LANES = 128
NB = 2
NG = 4
HW = 64
NT = HW // 4
NTILE = NT * NT
NPIX = HW * HW
NPOS = 36
NM = 6
PAD = 8
TAIL = (128, 64, 64)

SOFF = {(0, 1): 0, (0, 0): 8, (3, 1): 24, (3, 0): 32, (1, 0): 40, (1, 1): 48, (2, 0): 56, (2, 1): 64}
SROWS = 72


def _phase_scale(i, j):
    return R2 ** (3 - i - j) if (i + j) % 2 == 0 else 2.0 ** ((3 - i - j) // 2)


def _bt(p3m, p0, p1, p2, p3, p0n):
    t = p1 * 0.25
    er = p1 - p3
    e1 = p3 - t
    o1 = p2 - p0 * 0.25
    orr = p0 - p2
    e2 = er + er
    return [(p3m - t) - er, e1 + o1, e1 - o1, e2 + orr, e2 - orr, (p0n + orr) - p2 * 4.0]


def _gt(g0, g1, g2, c0=1.0 / 6.0, c1=R2 / 6.0):
    a0, a1, a2 = g0 * c0, g1 * c1, g2 * c0
    s = a0 + a2
    e1, er = s + a2, s + a0
    return [g0, e1 + a1, e1 - a1, er + a1, er - a1, g2]


def _at_even(m0, m1, m2, m3, m4):
    s1, sr = m1 + m2, m3 + m4
    return (m0 + s1) + sr, s1 * 4.0 + sr


def _at_odd(m1, m2, m3, m4, m5):
    d1, dr = m1 - m2, m3 - m4
    return (d1 + d1) + dr, (d1 * 8.0 + dr) + m5


def _unpack(w):
    return [lax.bitcast_convert_type(w << 16, F32), lax.bitcast_convert_type(w & np.uint32(0xFFFF0000), F32)]


def _pack(lo, hi):
    lo, hi = [lax.bitcast_convert_type(v.astype(BF16).astype(F32), U32) for v in (lo, hi)]
    return (lo >> 16) | hi


class _Moments:
    def __init__(self):
        self.pivot, self.sums = None, [None, None]

    def add(self, i, vs):
        if self.pivot is None:
            self.pivot = vs[0]
        ds = [v - self.pivot for v in vs]
        new = _tree_sum(ds), _tree_sum([d * d for d in ds])
        self.sums[i] = new if self.sums[i] is None else [a + b for a, b in zip(self.sums[i], new)]


def _tree_sum(vs):
    return vs[0] if len(vs) == 1 else _tree_sum(vs[:len(vs) // 2]) + _tree_sum(vs[len(vs) // 2:])


def _run(items):
    for f, _, _ in items:
        f()


def _overlap(dots, items):
    total = sum(rows for _, rows in dots)
    work = sum(cost for _, _, cost in items)
    done, issued, start, res = 0, 0, 0, None
    for f, gate, cost in items:
        t = int(done / work * 0.995 * total) // 8 * 8
        done += cost
        if gate is not None:
            while issued == 0 or t >= start + dots[issued - 1][1]:
                if issued:
                    start += dots[issued - 1][1]
                res = dots[issued][0]()
                issued += 1
            gate(res[t - start:t - start + 8])
        f()
    for f, _ in dots[issued:]:
        f()


def _kernel(x_hbm, t_hbm, g1_hbm, be1_hbm, w1_hbm, we_hbm, g2_hbm, be2_hbm, w2_hbm, o_hbm,
            xs, ob, ws, wes, ts, vecs, par, aff, cw, V, U, M, S, Hs, zs, sem):
    xu, ou, wu = xs.bitcast(U32), ob.bitcast(U32), ws.bitcast(U32)
    Vu, Uu = [v.bitcast(U32) for v in V], [u.bitcast(U32) for u in U]
    lo, hi, every = (0, 1), (2, 3), range(NG)
    slab = lambda g: pl.ds(g * LANES, LANES)

    def x_copy(b, g, r0=0, nr=NPIX):
        rows = pl.ds(r0, nr)
        return [(x_hbm.at[b, rows, slab(g)], xs.at[b * NG + g, rows])]

    def w_copy(c, ns, ks):
        w_hbm = (w1_hbm, w2_hbm)[c]
        return [(w_hbm.at[:, slab(n), slab(k)], ws.at[c * NG + k, :, slab(n), :]) for n in ns for k in ks]

    early = 3 * NPIX // 4
    loads = dict(
        w0=w_copy(0, (0,), lo), w1=w_copy(0, (1,), lo),
        x0a=[(g1_hbm, vecs[0]), (be1_hbm, vecs[1])] + x_copy(0, 0, 0, early), x0b=x_copy(0, 0, early, NPIX - early),
        x1a=x_copy(0, 1, 0, early), x1b=x_copy(0, 1, early, NPIX - early),
        bq=[(g2_hbm, vecs[2])], b0=[(be2_hbm, vecs[3]), (t_hbm, ts)],
        b1=x_copy(0, 2) + w_copy(0, hi, lo),
        b2=x_copy(0, 3) + w_copy(0, lo, hi),
        b3=w_copy(0, hi, hi) + x_copy(1, 0) + x_copy(1, 1) + [(we_hbm, wes)],
        b4=x_copy(1, 2) + x_copy(1, 3),
        b5=w_copy(1, every, every))
    osem = sem.at[len(loads)]

    def copies(name):
        return [pltpu.make_async_copy(src, dst, sem.at[list(loads).index(name)]) for src, dst in loads[name]]

    def start(*names):
        for name in names:
            for cp in copies(name):
                cp.start()

    def wait(name):
        for cp in copies(name):
            cp.wait()

    def write_out(b, g, r0, nr):
        rows = pl.ds(r0, nr)
        pltpu.make_async_copy(ob.at[b * NG + g, rows], o_hbm.at[b, rows, slab(g)], osem).start()

    start("w0", "w1", "x0a", "x0b", "x1a", "x1b")

    @pl.loop(0, 3)
    def _(i):
        zs[i] = i >> 2

    z0, z1 = zs[0], zs[1]

    def gate(ref, idx):
        def put(v):
            ref[idx] = v if ref.dtype == F32 else lax.bitcast_convert_type(v, U32)
        return put

    gate_x = gate(xu, (z1, pl.ds(NPIX // 2, 8)))
    gate_w = gate(wu, (z1, 0, pl.ds(NG * LANES // 2, 8)))
    gate_s = gate(S, (z1 + NT, 0, pl.ds(0, 8)))
    gate_c = gate(cw, z1 + 2)

    def new_block():
        @pl.loop(0, z1)
        def _(i):
            zs[2] = i

    def reload():
        for ref in Vu[:1] + Uu:
            ref[z1 + NPOS, 0, 0:8, :] = jnp.zeros((8, LANES), U32)

    def load_vecs(rows):
        for r in rows:
            v = vecs[r][...].astype(F32).reshape(1, NG * LANES)
            for g in every:
                par[g, r] = v[:, g * LANES:(g + 1) * LANES]

    def with_embedding(dots):
        parts, nparts = [], wes.shape[0] // LANES

        def part(i, f):
            t = 0.5 * ts[:, slab(i)].astype(F32)
            e = jnp.dot((t * (jnp.tanh(t) + 1.0)).astype(BF16), wes[slab(i), :], preferred_element_type=F32)
            parts.append(parts[-1] + e if i else e)
            if i == nparts - 1:
                load_vecs(hi)
                for g in every:
                    for b in range(NB):
                        par[g, 4 + b] = parts[-1][b:b + 1, g * LANES:(g + 1) * LANES]
            return f()

        first = [(lambda i=i, f=f: part(i - 1, f), nr) for i, (f, nr) in enumerate(dots) if 0 < i <= nparts]
        return dots[:1] + first + dots[nparts + 1:]

    def gn_finalize(slot, acc, gamma, beta, shift):
        s1, s2 = [a + b for a, b in zip(*acc.sums)]
        n = float(NPIX // 8)
        mean = lambda v: jnp.sum(jnp.sum(v, axis=0, keepdims=True), axis=1, keepdims=True) * (1.0 / (NPIX * LANES))
        mu = mean(s1 + (acc.pivot + shift) * n)
        d = (shift - mu) + acc.pivot
        var = mean(s2 + d * (2.0 * s1 + d * n))
        scale = (0.5 * gamma) * lax.rsqrt(jnp.maximum(var, 0.0) + EPS)
        aff[slot][0] = jnp.broadcast_to(scale, (8, LANES))
        aff[slot][1] = jnp.broadcast_to(0.5 * beta + (shift - mu) * scale, (8, LANES))

    def x_stats(b, g):
        acc = _Moments()

        def item(c):
            for r in range(8):
                acc.add(r & 1, _unpack(xu[b * NG + g, pl.ds((c * 8 + r) * 8, 8), :]))

        def fin():
            gn_finalize(b * NG + g, acc, par[g, 0], par[g, 1], jnp.zeros((1, LANES), F32))

        return [(lambda c=c: item(c), gate_x, 80) for c in range(32)] + [(fin, None, 40)]

    def in_transform(c, b, k, t0=0, t1=NT):
        slot = (c * NB + b) * NG + k
        held = {}

        def act(i, th, jp, e):
            if th in (-1, NT):
                return [jnp.zeros((8, LANES), F32)] * 2
            if c == 0:
                raw = _unpack(xu[b * NG + k, pl.ds((4 * th + i) * 32 + 2 * e + jp, 8, stride=4), :])
            else:
                raw = [Hs[b * NG + k][4 * i + 2 * jp + q, pl.ds(th * NT + 8 * e, 8), :] for q in range(2)]
            scale, bias = aff[slot][0], aff[slot][1]
            out = []
            for q in range(2):
                hz = raw[q] * scale + bias
                cz = _phase_scale(i, 2 * jp + q)
                t = jnp.tanh(hz)
                out.append(hz * (t + 1.0) if cz == 1.0 else hz * (t * cz + cz))
            return out

        def activate(th, jp, e):
            if th == t0:
                held[jp, e] = (act(3, th - 1, jp, e), act(0, th, jp, e))
            held["new"] = [act(i, th, jp, e) for i in (1, 2, 3)]

        def along_h(th, jp, e):
            (p3m, p0), (p1, p2, p3), p0n = held[jp, e], held["new"], act(0, th + 1, jp, e)
            for q in range(2):
                v = _bt(p3m[q], p0[q], p1[q], p2[q], p3[q], p0n[q])
                for xi in range(6):
                    S[th, xi, pl.ds(SOFF[2 * jp + q, e], 8), :] = v[xi]
            held[jp, e] = (p3, p0n)

        def along_w(th, xi):
            p = {je: S[th, xi, pl.ds(o, 8), :] for je, o in SOFF.items()}
            p0n = S[th, xi, pl.ds(SOFF[0, 0] + 1, 8), :]
            p3m = S[th, xi, pl.ds(SOFF[3, 1] - 1, 8), :]
            even = _bt(p3m, p[0, 0], p[1, 0], p[2, 0], p[3, 0], p[0, 1])
            odd = _bt(p[3, 0], p[0, 1], p[1, 1], p[2, 1], p[3, 1], p0n)
            for nu in range(6):
                V[b][xi * 6 + nu, k, pl.ds(th * NT, 8), :] = even[nu].astype(BF16)
                V[b][xi * 6 + nu, k, pl.ds(th * NT + 8, 8), :] = odd[nu].astype(BF16)

        src = gate_x if c == 0 else gate(Hs[b * NG + k], (z1, pl.ds(NTILE, 8)))
        items = []
        for c0 in range(t0, t1, 4):
            for jp in range(2):
                for e in range(2):
                    for th in range(c0, c0 + 4):
                        items.append((lambda a=(th, jp, e): activate(*a), src, (33 if c else 39) + 22 * (th == t0)))
                        items.append((lambda a=(th, jp, e): along_h(*a), src, 45 if c else 47))
            items += [(lambda a=(th, xi): along_w(*a), gate_s, 48) for th in range(c0, c0 + 4) for xi in range(6)]
        return items

    def w_transform(c, n, ks=every):
        held = {}

        def put(k, r, q, xi, nu, v):
            U[n][xi * 6 + nu, k, pl.ds(r * 16 + q * 8, 8), :] = v.astype(BF16)

        def along_h(k, r, q):
            raw = [wu[c * NG + k, t, pl.ds(n * 64 + r * 8, 8), :] for t in range(9)]
            g = [pltpu.bitcast(w, BF16).astype(F32)[8 * q:8 * q + 8] for w in raw]
            held["cols"] = cols = [_gt(g[l], g[3 + l], g[6 + l]) for l in range(3)]
            if q == 0:
                for xi in (0, 5):
                    for nu in (0, 5):
                        Uu[n][xi * 6 + nu, k, pl.ds(r * 8, 8), :] = raw[(xi // 5) * 6 + (nu // 5) * 2]
            for xi in range(1, 5):
                put(k, r, q, xi, 0, cols[0][xi])
                put(k, r, q, xi, 5, cols[2][xi])

        def along_w(k, r, q, xis):
            cols = held["cols"]
            c0, c1 = cw[0], cw[1]
            for xi in xis:
                u = _gt(cols[0][xi], cols[1][xi], cols[2][xi], c0, c1)
                for nu in range(1, 5):
                    put(k, r, q, xi, nu, u[nu])

        items = []
        for k in ks:
            for r in range(8):
                for q in range(2):
                    items.append((lambda a=(k, r, q): along_h(*a), gate_w, 55.25))
                    items += [(lambda a=(k, r, q, xis): along_w(*a), gate_c, 32.9) for xis in ((0, 5), (1, 2), (3, 4))]
        return items

    def nt_dot(lhs, rhs):
        return lax.dot_general(lhs, rhs, (((1,), (1,)), ((), ())), preferred_element_type=F32)

    def operand(ref, p, ks, rows=slice(None)):
        return jnp.concatenate([pltpu.bitcast(ref[p, k, rows, :], BF16) for k in ks], axis=1)

    def matmuls(s, r0=0, nr=NTILE, dst=None):
        def item(p):
            r = nt_dot(operand(Vu[s >> 2 & 1], p, every, pl.ds(r0 // 2, nr // 2)), operand(Uu[s & 3], p, every))
            M[s % NM if dst is None else dst][p, pl.ds(r0, nr), :] = r
            return r

        return [(lambda p=p: item(p), nr) for p in range(NPOS)]

    def matmuls_half(ns, ks, r0=0, nr=NTILE):
        def item(p):
            r = nt_dot(operand(Vu[0], p, ks, pl.ds(r0 // 2, nr // 2)),
                       jnp.concatenate([operand(Uu[n], p, ks) for n in ns], axis=0))
            for i, n in enumerate(ns):
                part = r[:, i * LANES:(i + 1) * LANES]
                if ks[0]:
                    part = part + M[n][p, pl.ds(r0, nr), :]
                M[n][p, pl.ds(r0, nr), :] = part
            return part

        return [(lambda p=p: item(p), nr) for p in range(NPOS)]

    def out_transform(s, r0=0, nr=NTILE, src=None, piece=None):
        c, b, n = s >> 3, s >> 2 & 1, s & 3
        src = M[s % NM if src is None else src]
        piece = piece or nr
        acc, held = _Moments(), {}

        def along_h(tv, odd, nus):
            for nu in nus:
                m = [src[z0 + xi * 6 + nu, pl.ds(tv * 8, 8), :] for xi in range(odd, 5 + odd)]
                held[nu] = (_at_odd if odd else _at_even)(*m)

        def along_w(tv, odd):
            for q in range(2):
                i = odd + 2 * q
                m = [held[nu][q] for nu in range(6)]
                (y0, y2), (y1, y3) = _at_even(*m[:5]), _at_odd(*m[1:])
                y = [z if _phase_scale(i, j) == 1.0 else z * _phase_scale(i, j) for j, z in enumerate((y0, y1, y2, y3))]
                if c == 0:
                    for j in range(4):
                        Hs[b * NG + n][4 * i + j, pl.ds(tv * 8, 8), :] = y[j]
                    acc.add(q, y)
                else:
                    for jp in range(2):
                        sl = pl.ds((4 * (tv // 2) + i) * 32 + 2 * (tv % 2) + jp, 8, stride=4)
                        u, v = _unpack(xu[b * NG + n, sl, :])
                        ou[b * NG + n, sl, :] = _pack(u + y[2 * jp], v + y[2 * jp + 1])

        def fin(end):
            if c == 0:
                gn_finalize((NB + b) * NG + n, acc, par[n, 2], par[n, 3], par[n, 4 + b])
            else:
                write_out(b, n, (end - piece) * 16, piece * 16)

        g = gate(src, (z1, pl.ds(NTILE, 8)))
        items = []
        for tv in range(r0 // 8, (r0 + nr) // 8):
            for odd in range(2):
                items += [(lambda a=(tv, odd, nus): along_h(*a), g, 21) for nus in ((0, 1, 2), (3, 4, 5))]
                items += [(lambda a=(tv, odd): along_w(*a), None, 72 if c else 64)]
            if (tv * 8 + 8 - r0) % piece == 0:
                items.append((lambda end=tv * 8 + 8: fin(end), None, 40))
        return items

    ST, IN, WT, MM, MH, OUT = x_stats, in_transform, w_transform, matmuls, matmuls_half, out_transform
    H, T2 = NT // 2, NTILE // 2

    cw[0] = jnp.full((8, LANES), 1.0 / 6.0, F32)
    cw[1] = jnp.full((8, LANES), R2 / 6.0, F32)
    S[:, :, pl.ds(16, 8), :] = jnp.zeros((NT + 1, 6, 8, LANES), F32)

    wait("w0")
    _run(WT(0, 0, lo))
    wait("w1")
    _run(WT(0, 1, lo))
    wait("x0a")
    start("b0", "bq", "b1")
    load_vecs(lo)
    stats = ST(0, 0)
    _run(stats[:24])
    wait("x0b")
    first = IN(0, 0, 0, 0, H)
    _run(stats[24:] + first[:-24])
    stats = ST(0, 1)
    wait("x1a")
    _run(stats[:24])
    wait("x1b")
    start("b2")
    _run(stats[24:] + first[-24:] + IN(0, 0, 1, 0, 4))

    wait("b0")
    _overlap(MH(lo, lo, 0, 64), IN(0, 0, 1, 4, H) + IN(0, 0, 0, H, 12))
    wait("bq")
    _overlap(MH(lo, lo, 64, 64), IN(0, 0, 0, 12, NT) + IN(0, 0, 1, H, NT))
    reload()
    wait("b1")
    start("b3")
    _overlap(MH(lo, lo, T2, T2), ST(0, 2) + WT(0, 2, lo) + WT(0, 3, lo))
    reload()
    wait("b2")
    start("b4")
    _overlap(MH(hi, lo), ST(0, 3) + WT(0, 0, hi) + IN(0, 0, 2, 0, H) + IN(0, 0, 3, 0, H) + WT(0, 1, hi))

    new_block()
    wait("b3")
    start("b5")
    _overlap(MH(lo, hi, 0, T2), ST(1, 0) + IN(0, 0, 2, H, NT) + IN(0, 0, 3, H, NT))
    _overlap(MH(lo, hi, T2, T2), ST(1, 1) + WT(0, 2, hi) + WT(0, 3, hi))

    new_block()
    wait("b4")
    out0, out2 = OUT(0), OUT(2)
    mid = len(out0) // 2
    _overlap(with_embedding(MH(hi, hi)), sum([ST(1, 2), ST(1, 3)] + [IN(0, 1, k, 0, H) for k in every], []))
    _overlap(MM(4, 0, T2) + MM(5, 0, T2), sum([IN(0, 1, k, H, NT) for k in every], []) + out0[:mid])

    new_block()
    wait("b5")
    _overlap(MM(4, T2, T2) + MM(5, T2, T2), out0[mid:] + OUT(1) + IN(1, 0, 0) + out2[:mid])
    _overlap(MM(6), out2[mid:] + IN(1, 0, 1) + IN(1, 0, 2, 0, H) + WT(1, 0, (0, 1, 2)))

    new_block()
    _overlap(MM(7), OUT(3) + IN(1, 0, 2, H, NT) + IN(1, 0, 3) + WT(1, 0, (3,)))
    _overlap(MM(8), OUT(4) + OUT(5) + WT(1, 1))

    new_block()
    _overlap(MM(9), IN(1, 1, 0) + IN(1, 1, 1, 0, H) + WT(1, 2))
    _overlap(MM(10), OUT(6) + IN(1, 1, 1, H, NT) + IN(1, 1, 2, 0, 4) + WT(1, 3))

    new_block()
    _overlap(MM(11), OUT(7) + IN(1, 1, 2, 4, NT) + IN(1, 1, 3))
    _overlap(MM(12), OUT(8) + OUT(9))
    dots, items = MM(13), OUT(10) + OUT(11)
    cut = 5 * len(items) // 12
    _overlap(dots[:15], items[:cut])

    new_block()
    _overlap(dots[15:], items[cut:])
    _overlap(MM(14), OUT(12) + OUT(13))
    items, r0 = OUT(14), 0
    for i, nr in enumerate(TAIL):
        _overlap(MM(15, r0, nr, (15 + i) % NM), items)
        items = OUT(15, r0, nr, (15 + i) % NM, NT if i == len(TAIL) - 1 else None)
        r0 += nr
    _run(items)
    pltpu.make_async_copy(ob, ob, osem).wait()


@jax.jit
def pallas_standalone__adm_resblock__diffusion_kernel(
    x: jax.Array,
    t_emb: jax.Array,
    g1: jax.Array,
    be1: jax.Array,
    w1: jax.Array,
    w_emb: jax.Array,
    g2: jax.Array,
    be2: jax.Array,
    w2: jax.Array,
):
    B, C, H, W = x.shape
    E = t_emb.shape[1]
    assert (B, C, H, W) == (NB, NG * LANES, HW, HW)
    xl = x.transpose(0, 2, 3, 1).reshape(B, NPIX, C)
    w1l = w1.transpose(2, 3, 0, 1).reshape(9, C, C)
    w2l = w2.transpose(2, 3, 0, 1).reshape(9, C, C)
    hbm = pl.BlockSpec(memory_space=pltpu.HBM)
    out = pl.pallas_call(
        _kernel,
        out_shape=jax.ShapeDtypeStruct((B, NPIX, C), x.dtype),
        in_specs=[hbm] * 9,
        out_specs=hbm,
        scratch_shapes=[
            pltpu.VMEM((B * NG, NPIX + 2 * PAD, LANES), BF16),
            pltpu.VMEM((B * NG, NPIX, LANES), BF16),
            pltpu.VMEM((2 * NG, 9, C + 2 * PAD, LANES), BF16),
            pltpu.VMEM((E, C), BF16),
            pltpu.VMEM((B, E), BF16),
            [pltpu.VMEM((C,), BF16)] * 4,
            pltpu.VMEM((NG, 4 + B, 1, LANES), F32),
            [pltpu.VMEM((2, 8, LANES), F32)] * (2 * B * NG),
            pltpu.VMEM((3, 8, LANES), F32),
            [pltpu.VMEM((NPOS + 1, NG, NTILE, LANES), BF16)] * B,
            [pltpu.VMEM((NPOS + 1, NG, LANES, LANES), BF16)] * NG,
            [pltpu.VMEM((NPOS, NTILE + PAD, LANES), F32)] * NM,
            pltpu.VMEM((NT + 1, 6, SROWS, LANES), F32),
            [pltpu.VMEM((16, NTILE + PAD, LANES), F32)] * (B * NG),
            pltpu.SMEM((3,), jnp.int32),
            pltpu.SemaphoreType.DMA((14,)),
        ],
        compiler_params=pltpu.CompilerParams(vmem_limit_bytes=124 * 2 ** 20),
        name="adm_resblock",
    )(xl, t_emb, g1, be1, w1l, w_emb, g2, be2, w2l)
    return out.reshape(B, H, W, C).transpose(0, 3, 1, 2)
```

```python
import numpy as np
import jax
import jax.numpy as jnp
from jax import lax
import jax.experimental.pallas as pl
import jax.experimental.pallas.tpu as pltpu

F32, BF16, U32 = jnp.float32, jnp.bfloat16, jnp.uint32
R2 = 2.0 ** 0.5
EPS = 1e-5
LANES = 128
NB = 2
NG = 4
HW = 64
NT = HW // 4
NTILE = NT * NT
NPIX = HW * HW
NPOS = 36
NM = 6
PAD = 8

SOFF = {(0, 1): 0, (0, 0): 8, (3, 1): 24, (3, 0): 32, (1, 0): 40, (1, 1): 48, (2, 0): 56, (2, 1): 64}
SROWS = 72


def _phase_scale(i, j):
    return R2 ** (3 - i - j) if (i + j) % 2 == 0 else 2.0 ** ((3 - i - j) // 2)


def _bt(p3m, p0, p1, p2, p3, p0n):
    t = p1 * 0.25
    er = p1 - p3
    e1 = p3 - t
    o1 = p2 - p0 * 0.25
    orr = p0 - p2
    e2 = er + er
    return [(p3m - t) - er, e1 + o1, e1 - o1, e2 + orr, e2 - orr, (p0n + orr) - p2 * 4.0]


def _gt(g0, g1, g2, c0=1.0 / 6.0, c1=R2 / 6.0):
    a0, a1, a2 = g0 * c0, g1 * c1, g2 * c0
    s = a0 + a2
    e1, er = s + a2, s + a0
    return [g0, e1 + a1, e1 - a1, er + a1, er - a1, g2]


def _at_even(m0, m1, m2, m3, m4):
    s1, sr = m1 + m2, m3 + m4
    return (m0 + s1) + sr, s1 * 4.0 + sr


def _at_odd(m1, m2, m3, m4, m5):
    d1, dr = m1 - m2, m3 - m4
    return (d1 + d1) + dr, (d1 * 8.0 + dr) + m5


def _unpack(w):
    return [lax.bitcast_convert_type(w << 16, F32), lax.bitcast_convert_type(w & np.uint32(0xFFFF0000), F32)]


def _pack(lo, hi):
    lo, hi = [lax.bitcast_convert_type(v.astype(BF16).astype(F32), U32) for v in (lo, hi)]
    return (lo >> 16) | hi


class _Moments:
    def __init__(self):
        self.pivot, self.sums = None, [None, None]

    def add(self, i, vs):
        if self.pivot is None:
            self.pivot = vs[0]
        ds = [v - self.pivot for v in vs]
        new = _tree_sum(ds), _tree_sum([d * d for d in ds])
        self.sums[i] = new if self.sums[i] is None else [a + b for a, b in zip(self.sums[i], new)]


def _tree_sum(vs):
    return vs[0] if len(vs) == 1 else _tree_sum(vs[:len(vs) // 2]) + _tree_sum(vs[len(vs) // 2:])


def _run(items):
    for f, _, _ in items:
        f()


def _overlap(dots, items):
    total = sum(rows for _, rows in dots)
    work = sum(cost for _, _, cost in items)
    done, issued, start, res = 0, 0, 0, None
    for f, gate, cost in items:
        t = int(done / work * 0.995 * total) // 8 * 8
        done += cost
        if gate is not None:
            while issued == 0 or t >= start + dots[issued - 1][1]:
                if issued:
                    start += dots[issued - 1][1]
                res = dots[issued][0]()
                issued += 1
            gate(res[t - start:t - start + 8])
        f()
    for f, _ in dots[issued:]:
        f()


def _kernel(x_hbm, t_hbm, g1_hbm, be1_hbm, w1_hbm, we_hbm, g2_hbm, be2_hbm, w2_hbm, o_hbm,
            xs, ob, ws, wes, ts, vecs, par, aff, cw, V, U, M, S, Hs, zs, sem):
    xu, ou, wu = xs.bitcast(U32), ob.bitcast(U32), ws.bitcast(U32)
    Vu, Uu = [v.bitcast(U32) for v in V], [u.bitcast(U32) for u in U]
    lo, hi, every = (0, 1), (2, 3), range(NG)
    slab = lambda g: pl.ds(g * LANES, LANES)

    def x_copy(b, g, r0=0, nr=NPIX):
        rows = pl.ds(r0, nr)
        return [(x_hbm.at[b, rows, slab(g)], xs.at[b * NG + g, rows])]

    def w_copy(c, ns, ks):
        w_hbm = (w1_hbm, w2_hbm)[c]
        return [(w_hbm.at[:, slab(n), slab(k)], ws.at[c * NG + k, :, slab(n), :]) for n in ns for k in ks]

    early = 3 * NPIX // 4
    loads = dict(
        w0=w_copy(0, (0,), lo), w1=w_copy(0, (1,), lo),
        x0a=[(g1_hbm, vecs[0]), (be1_hbm, vecs[1])] + x_copy(0, 0, 0, early), x0b=x_copy(0, 0, early, NPIX - early),
        x1a=x_copy(0, 1, 0, early), x1b=x_copy(0, 1, early, NPIX - early),
        b0=[(g2_hbm, vecs[2]), (be2_hbm, vecs[3]), (t_hbm, ts)],
        b1=x_copy(0, 2) + w_copy(0, hi, lo),
        b2=x_copy(0, 3) + w_copy(0, lo, hi),
        b3=w_copy(0, hi, hi) + x_copy(1, 0) + x_copy(1, 1) + [(we_hbm, wes)],
        b4=x_copy(1, 2) + x_copy(1, 3),
        b5=w_copy(1, every, every))
    osem = sem.at[len(loads)]

    def copies(name):
        return [pltpu.make_async_copy(src, dst, sem.at[list(loads).index(name)]) for src, dst in loads[name]]

    def start(*names):
        for name in names:
            for cp in copies(name):
                cp.start()

    def wait(name):
        for cp in copies(name):
            cp.wait()

    def write_out(b, g, r0, nr):
        rows = pl.ds(r0, nr)
        pltpu.make_async_copy(ob.at[b * NG + g, rows], o_hbm.at[b, rows, slab(g)], osem).start()

    start("w0", "w1", "x0a", "x0b", "x1a", "x1b")

    @pl.loop(0, 3)
    def _(i):
        zs[i] = i >> 2

    z0, z1 = zs[0], zs[1]

    def gate(ref, idx):
        def put(v):
            ref[idx] = v if ref.dtype == F32 else lax.bitcast_convert_type(v, U32)
        return put

    gate_x = gate(xu, (z1, pl.ds(NPIX // 2, 8)))
    gate_w = gate(wu, (z1, 0, pl.ds(NG * LANES // 2, 8)))
    gate_s = gate(S, (z1 + NT, 0, pl.ds(0, 8)))
    gate_c = gate(cw, z1 + 2)

    def new_block():
        @pl.loop(0, z1)
        def _(i):
            zs[2] = i

    def reload():
        for ref in Vu[:1] + Uu:
            ref[z1 + NPOS, 0, 0:8, :] = jnp.zeros((8, LANES), U32)

    def load_vecs(rows):
        for r in rows:
            v = vecs[r][...].astype(F32).reshape(1, NG * LANES)
            for g in every:
                par[g, r] = v[:, g * LANES:(g + 1) * LANES]

    def with_embedding(dots):
        parts, nparts = [], wes.shape[0] // LANES

        def part(i, f):
            t = 0.5 * ts[:, slab(i)].astype(F32)
            e = jnp.dot((t * (jnp.tanh(t) + 1.0)).astype(BF16), wes[slab(i), :], preferred_element_type=F32)
            parts.append(parts[-1] + e if i else e)
            if i == nparts - 1:
                load_vecs(hi)
                for g in every:
                    for b in range(NB):
                        par[g, 4 + b] = parts[-1][b:b + 1, g * LANES:(g + 1) * LANES]
            return f()

        first = [(lambda i=i, f=f: part(i - 1, f), nr) for i, (f, nr) in enumerate(dots) if 0 < i <= nparts]
        return dots[:1] + first + dots[nparts + 1:]

    def gn_finalize(slot, acc, gamma, beta, shift):
        s1, s2 = [a + b for a, b in zip(*acc.sums)]
        n = float(NPIX // 8)
        mean = lambda v: jnp.sum(jnp.sum(v, axis=0, keepdims=True), axis=1, keepdims=True) * (1.0 / (NPIX * LANES))
        mu = mean(s1 + (acc.pivot + shift) * n)
        d = (shift - mu) + acc.pivot
        var = mean(s2 + d * (2.0 * s1 + d * n))
        scale = (0.5 * gamma) * lax.rsqrt(jnp.maximum(var, 0.0) + EPS)
        aff[slot][0] = jnp.broadcast_to(scale, (8, LANES))
        aff[slot][1] = jnp.broadcast_to(0.5 * beta + (shift - mu) * scale, (8, LANES))

    def x_stats(b, g):
        acc = _Moments()

        def item(c):
            for r in range(8):
                acc.add(r & 1, _unpack(xu[b * NG + g, pl.ds((c * 8 + r) * 8, 8), :]))

        def fin():
            gn_finalize(b * NG + g, acc, par[g, 0], par[g, 1], jnp.zeros((1, LANES), F32))

        return [(lambda c=c: item(c), gate_x, 80) for c in range(32)] + [(fin, None, 40)]

    def in_transform(c, b, k, t0=0, t1=NT):
        slot = (c * NB + b) * NG + k
        held = {}

        def act(i, th, jp, e):
            if th in (-1, NT):
                return [jnp.zeros((8, LANES), F32)] * 2
            if c == 0:
                raw = _unpack(xu[b * NG + k, pl.ds((4 * th + i) * 32 + 2 * e + jp, 8, stride=4), :])
            else:
                raw = [Hs[b * NG + k][4 * i + 2 * jp + q, pl.ds(th * NT + 8 * e, 8), :] for q in range(2)]
            scale, bias = aff[slot][0], aff[slot][1]
            out = []
            for q in range(2):
                hz = raw[q] * scale + bias
                cz = _phase_scale(i, 2 * jp + q)
                t = jnp.tanh(hz)
                out.append(hz * (t + 1.0) if cz == 1.0 else hz * (t * cz + cz))
            return out

        def activate(th, jp, e):
            if th == t0:
                held[jp, e] = (act(3, th - 1, jp, e), act(0, th, jp, e))
            held["new"] = [act(i, th, jp, e) for i in (1, 2, 3)]

        def along_h(th, jp, e):
            (p3m, p0), (p1, p2, p3), p0n = held[jp, e], held["new"], act(0, th + 1, jp, e)
            for q in range(2):
                v = _bt(p3m[q], p0[q], p1[q], p2[q], p3[q], p0n[q])
                for xi in range(6):
                    S[th, xi, pl.ds(SOFF[2 * jp + q, e], 8), :] = v[xi]
            held[jp, e] = (p3, p0n)

        def along_w(th, xi):
            p = {je: S[th, xi, pl.ds(o, 8), :] for je, o in SOFF.items()}
            p0n = S[th, xi, pl.ds(SOFF[0, 0] + 1, 8), :]
            p3m = S[th, xi, pl.ds(SOFF[3, 1] - 1, 8), :]
            even = _bt(p3m, p[0, 0], p[1, 0], p[2, 0], p[3, 0], p[0, 1])
            odd = _bt(p[3, 0], p[0, 1], p[1, 1], p[2, 1], p[3, 1], p0n)
            for nu in range(6):
                V[b][xi * 6 + nu, k, pl.ds(th * NT, 8), :] = even[nu].astype(BF16)
                V[b][xi * 6 + nu, k, pl.ds(th * NT + 8, 8), :] = odd[nu].astype(BF16)

        src = gate_x if c == 0 else gate(Hs[b * NG + k], (z1, pl.ds(NTILE, 8)))
        items = []
        for c0 in range(t0, t1, 4):
            for jp in range(2):
                for e in range(2):
                    for th in range(c0, c0 + 4):
                        items.append((lambda a=(th, jp, e): activate(*a), src, (33 if c else 39) + 22 * (th == t0)))
                        items.append((lambda a=(th, jp, e): along_h(*a), src, 45 if c else 47))
            items += [(lambda a=(th, xi): along_w(*a), gate_s, 48) for th in range(c0, c0 + 4) for xi in range(6)]
        return items

    def w_transform(c, n, ks=every):
        held = {}

        def put(k, r, q, xi, nu, v):
            U[n][xi * 6 + nu, k, pl.ds(r * 16 + q * 8, 8), :] = v.astype(BF16)

        def along_h(k, r, q):
            raw = [wu[c * NG + k, t, pl.ds(n * 64 + r * 8, 8), :] for t in range(9)]
            g = [pltpu.bitcast(w, BF16).astype(F32)[8 * q:8 * q + 8] for w in raw]
            held["cols"] = cols = [_gt(g[l], g[3 + l], g[6 + l]) for l in range(3)]
            if q == 0:
                for xi in (0, 5):
                    for nu in (0, 5):
                        Uu[n][xi * 6 + nu, k, pl.ds(r * 8, 8), :] = raw[(xi // 5) * 6 + (nu // 5) * 2]
            for xi in range(1, 5):
                put(k, r, q, xi, 0, cols[0][xi])
                put(k, r, q, xi, 5, cols[2][xi])

        def along_w(k, r, q, xis):
            cols = held["cols"]
            c0, c1 = cw[0], cw[1]
            for xi in xis:
                u = _gt(cols[0][xi], cols[1][xi], cols[2][xi], c0, c1)
                for nu in range(1, 5):
                    put(k, r, q, xi, nu, u[nu])

        items = []
        for k in ks:
            for r in range(8):
                for q in range(2):
                    items.append((lambda a=(k, r, q): along_h(*a), gate_w, 55.25))
                    items += [(lambda a=(k, r, q, xis): along_w(*a), gate_c, 32.9) for xis in ((0, 5), (1, 2), (3, 4))]
        return items

    def nt_dot(lhs, rhs):
        return lax.dot_general(lhs, rhs, (((1,), (1,)), ((), ())), preferred_element_type=F32)

    def operand(ref, p, ks, rows=slice(None)):
        return jnp.concatenate([pltpu.bitcast(ref[p, k, rows, :], BF16) for k in ks], axis=1)

    def matmuls(s, r0=0, nr=NTILE, dst=None):
        def item(p):
            r = nt_dot(operand(Vu[s >> 2 & 1], p, every, pl.ds(r0 // 2, nr // 2)), operand(Uu[s & 3], p, every))
            M[s % NM if dst is None else dst][p, pl.ds(r0, nr), :] = r
            return r

        return [(lambda p=p: item(p), nr) for p in range(NPOS)]

    def matmuls_half(ns, ks, r0=0, nr=NTILE):
        def item(p):
            r = nt_dot(operand(Vu[0], p, ks, pl.ds(r0 // 2, nr // 2)),
                       jnp.concatenate([operand(Uu[n], p, ks) for n in ns], axis=0))
            for i, n in enumerate(ns):
                part = r[:, i * LANES:(i + 1) * LANES]
                if ks[0]:
                    part = part + M[n][p, pl.ds(r0, nr), :]
                M[n][p, pl.ds(r0, nr), :] = part
            return part

        return [(lambda p=p: item(p), nr) for p in range(NPOS)]

    def out_transform(s, r0=0, nr=NTILE, src=None, piece=None, src0=None, odds=(0, 1)):
        c, b, n = s >> 3, s >> 2 & 1, s & 3
        src = M[s % NM if src is None else src]
        src0 = src if src0 is None else M[src0]
        piece = piece or nr
        acc, held = _Moments(), {}

        def along_h(tv, odd, nus):
            for nu in nus:
                m = [(src if xi else src0)[z0 + xi * 6 + nu, pl.ds(tv * 8, 8), :] for xi in range(odd, 5 + odd)]
                held[nu] = (_at_odd if odd else _at_even)(*m)

        def along_w(tv, odd):
            for q in range(2):
                i = odd + 2 * q
                m = [held[nu][q] for nu in range(6)]
                (y0, y2), (y1, y3) = _at_even(*m[:5]), _at_odd(*m[1:])
                y = [z if _phase_scale(i, j) == 1.0 else z * _phase_scale(i, j) for j, z in enumerate((y0, y1, y2, y3))]
                if c == 0:
                    for j in range(4):
                        Hs[b * NG + n][4 * i + j, pl.ds(tv * 8, 8), :] = y[j]
                    acc.add(q, y)
                else:
                    for jp in range(2):
                        sl = pl.ds((4 * (tv // 2) + i) * 32 + 2 * (tv % 2) + jp, 8, stride=4)
                        u, v = _unpack(xu[b * NG + n, sl, :])
                        ou[b * NG + n, sl, :] = _pack(u + y[2 * jp], v + y[2 * jp + 1])

        def fin(end):
            if c == 0:
                gn_finalize((NB + b) * NG + n, acc, par[n, 2], par[n, 3], par[n, 4 + b])
            else:
                write_out(b, n, (end - piece) * 16, piece * 16)

        g = gate(src, (z1, pl.ds(NTILE, 8)))
        items = []
        for tv in range(r0 // 8, (r0 + nr) // 8):
            for odd in odds:
                items += [(lambda a=(tv, odd, nus): along_h(*a), g, 21) for nus in ((0, 1, 2), (3, 4, 5))]
                items += [(lambda a=(tv, odd): along_w(*a), None, 72 if c else 64)]
            if 0 in odds and (tv * 8 + 8 - r0) % piece == 0:
                items.append((lambda end=tv * 8 + 8: fin(end), None, 40))
        return items

    ST, IN, WT, MM, MH, OUT = x_stats, in_transform, w_transform, matmuls, matmuls_half, out_transform
    H, T2 = NT // 2, NTILE // 2

    cw[0] = jnp.full((8, LANES), 1.0 / 6.0, F32)
    cw[1] = jnp.full((8, LANES), R2 / 6.0, F32)
    S[:, :, pl.ds(16, 8), :] = jnp.zeros((NT + 1, 6, 8, LANES), F32)

    wait("w0")
    _run(WT(0, 0, lo))
    wait("w1")
    _run(WT(0, 1, lo))
    wait("x0a")
    start("b0", "b1")
    load_vecs(lo)
    stats = ST(0, 0)
    _run(stats[:24])
    wait("x0b")
    first = IN(0, 0, 0, 0, H)
    _run(stats[24:] + first[:-24])
    stats = ST(0, 1)
    wait("x1a")
    _run(stats[:24])
    wait("x1b")
    start("b2")
    _run(stats[24:] + first[-24:] + IN(0, 0, 1, 0, 4))

    wait("b0")
    _overlap(MH(lo, lo, 0, 64), IN(0, 0, 1, 4, H) + IN(0, 0, 0, H, 12))
    _overlap(MH(lo, lo, 64, 64), IN(0, 0, 0, 12, NT) + IN(0, 0, 1, H, NT))
    reload()
    wait("b1")
    start("b3")
    _overlap(MH(lo, lo, T2, T2), ST(0, 2) + WT(0, 2, lo) + WT(0, 3, lo))
    reload()
    wait("b2")
    start("b4")
    _overlap(MH(hi, lo), ST(0, 3) + WT(0, 0, hi) + IN(0, 0, 2, 0, H) + IN(0, 0, 3, 0, H) + WT(0, 1, hi))

    new_block()
    wait("b3")
    start("b5")
    _overlap(MH(lo, hi, 0, T2), ST(1, 0) + IN(0, 0, 2, H, NT) + IN(0, 0, 3, H, NT))
    _overlap(MH(lo, hi, T2, T2), ST(1, 1) + WT(0, 2, hi) + WT(0, 3, hi))

    new_block()
    wait("b4")
    out0, out2 = OUT(0), OUT(2)
    mid = len(out0) // 2
    _overlap(with_embedding(MH(hi, hi)), sum([ST(1, 2), ST(1, 3)] + [IN(0, 1, k, 0, H) for k in every], []))
    _overlap(MM(4, 0, T2) + MM(5, 0, T2), sum([IN(0, 1, k, H, NT) for k in every], []) + out0[:mid])

    new_block()
    wait("b5")
    _overlap(MM(4, T2, T2) + MM(5, T2, T2), out0[mid:] + OUT(1) + IN(1, 0, 0) + out2[:mid])
    _overlap(MM(6), out2[mid:] + IN(1, 0, 1) + IN(1, 0, 2, 0, H) + WT(1, 0, (0, 1, 2)))

    new_block()
    _overlap(MM(7), OUT(3) + IN(1, 0, 2, H, NT) + IN(1, 0, 3) + WT(1, 0, (3,)))
    _overlap(MM(8), OUT(4) + OUT(5) + WT(1, 1))

    new_block()
    _overlap(MM(9), IN(1, 1, 0) + IN(1, 1, 1, 0, H) + WT(1, 2))
    _overlap(MM(10), OUT(6) + IN(1, 1, 1, H, NT) + IN(1, 1, 2, 0, 4) + WT(1, 3))

    new_block()
    _overlap(MM(11), OUT(7) + IN(1, 1, 2, 4, NT) + IN(1, 1, 3))
    _overlap(MM(12), OUT(8) + OUT(9))
    dots, items = MM(13), OUT(10) + OUT(11)
    cut = 5 * len(items) // 12
    _overlap(dots[:15], items[:cut])

    new_block()
    _overlap(dots[15:], items[cut:])
    _overlap(MM(14), OUT(12) + OUT(13))
    _overlap(MM(15, 0, 128, 3), OUT(14))
    _overlap(MM(15, 128, 64, 4), OUT(15, 0, 128, 3))
    _overlap(MM(15, 192, 64, 5)[6:], OUT(15, 128, 64, 4))
    for f, _ in MM(15, 192, 64, 0)[:6]:
        f()
    _run(OUT(15, 192, 64, 5, odds=(1,)))
    _run(OUT(15, 192, 64, 5, NT, 0, odds=(0,)))
    written = ob.at[:, pl.ds(0, NPIX)]
    pltpu.make_async_copy(written, written, osem).wait()


@jax.jit
def pallas_standalone__adm_resblock__diffusion_kernel(
    x: jax.Array,
    t_emb: jax.Array,
    g1: jax.Array,
    be1: jax.Array,
    w1: jax.Array,
    w_emb: jax.Array,
    g2: jax.Array,
    be2: jax.Array,
    w2: jax.Array,
):
    B, C, H, W = x.shape
    E = t_emb.shape[1]
    assert (B, C, H, W) == (NB, NG * LANES, HW, HW)
    xl = x.transpose(0, 2, 3, 1).reshape(B, NPIX, C)
    w1l = w1.transpose(2, 3, 0, 1).reshape(9, C, C)
    w2l = w2.transpose(2, 3, 0, 1).reshape(9, C, C)
    hbm = pl.BlockSpec(memory_space=pltpu.HBM)
    out = pl.pallas_call(
        _kernel,
        out_shape=jax.ShapeDtypeStruct((B, NPIX, C), x.dtype),
        in_specs=[hbm] * 9,
        out_specs=hbm,
        scratch_shapes=[
            pltpu.VMEM((B * NG, NPIX + 2 * PAD, LANES), BF16),
            pltpu.VMEM((B * NG, NPIX + 2 * PAD, LANES), BF16),
            pltpu.VMEM((2 * NG, 9, C + 2 * PAD, LANES), BF16),
            pltpu.VMEM((E, C), BF16),
            pltpu.VMEM((B, E), BF16),
            [pltpu.VMEM((C,), BF16)] * 4,
            pltpu.VMEM((NG, 4 + B, 1, LANES), F32),
            [pltpu.VMEM((2, 8, LANES), F32)] * (2 * B * NG),
            pltpu.VMEM((3, 8, LANES), F32),
            [pltpu.VMEM((NPOS + 1, NG, NTILE, LANES), BF16)] * B,
            [pltpu.VMEM((NPOS + 1, NG, LANES, LANES), BF16)] * NG,
            [pltpu.VMEM((NPOS, NTILE + PAD, LANES), F32)] * NM,
            pltpu.VMEM((NT + 1, 6, SROWS, LANES), F32),
            [pltpu.VMEM((16, NTILE + PAD, LANES), F32)] * (B * NG),
            pltpu.SMEM((3,), jnp.int32),
            pltpu.SemaphoreType.DMA((13,)),
        ],
        compiler_params=pltpu.CompilerParams(vmem_limit_bytes=124 * 2 ** 20),
        name="adm_resblock",
    )(xl, t_emb, g1, be1, w1l, w_emb, g2, be2, w2l)
    return out.reshape(B, H, W, C).transpose(0, 3, 1, 2)
```
